```python
import os as _os
_os.environ.setdefault("JAX_PLATFORMS", "cpu")
import jax
import jax.numpy as jnp

def _softmax(x, axis=-1):
    return jax.nn.softmax(x, axis=axis)
def _gelu(x):
    return jax.nn.gelu(x, approximate=True)
def _silu(x):
    return jax.nn.silu(x)
def _sigmoid(x):
    return jax.nn.sigmoid(x)
def _layernorm(x, axis=-1, eps=1e-5):
    m = jnp.mean(x, axis=axis, keepdims=True)
    v = jnp.var(x, axis=axis, keepdims=True)
    return (x - m) / jnp.sqrt(v + eps)
def _scatter_add(tgt, idx, src, axis=0):
    return tgt.at[idx].add(src)
def _segment_sum(src, seg, n):
    return jax.ops.segment_sum(src, seg, n)
class _Rng:
    def __init__(self, key):
        self._k = key
    def _next(self):
        self._k, sub = jax.random.split(self._k)
        return sub
    def normal(self, shape):
        return jax.random.normal(self._next(), shape, dtype=jnp.bfloat16)
    def randint(self, lo, hi, shape):
        return jax.random.randint(self._next(), shape, lo, hi, dtype=jnp.int32)
    def uniform(self, shape, lo=0.0, hi=1.0):
        return jax.random.uniform(self._next(), shape, jnp.bfloat16, lo, hi)
    def permutation(self, n):
        return jax.random.permutation(self._next(), n)


kernel_name = 'concat_heads__gqa_block_cached__gqa_block_cached__near_ridge'

def setup_inputs():
    _rng = _Rng(jax.random.key(int.from_bytes(__import__("os").urandom(4), "little")))
    _w = (lambda a: (lambda t: t.astype(jnp.bfloat16) if jnp.issubdtype(t.dtype, jnp.floating) else t)(jnp.asarray(a)))
    def _A_setup():
        B, Sq, D = 32, 48, 512
        Hq, Hkv, Sk, Dh = 32, 32, 48, 128
        assert Hq % Hkv == 0, (Hq, Hkv)
        return {
            "x": _w((lambda *s: _rng.normal(s) * 0.8)(B, Sq, D)),
            "k_cache": _w((lambda *s: _rng.normal(s) * 0.8)(B, Hkv, Sk, Dh)),
            "v_cache": _w((lambda *s: _rng.normal(s) * 0.05)(B, Hkv, Sk, Dh)),
            "wq": _w((lambda *s: _rng.normal(s) * 0.8)(D, Hq * Dh) * (D ** -0.5)),
            "wo": _w((lambda *s: _rng.normal(s) * 0.05)(Hq * Dh, D) * ((Hq * Dh) ** -0.5)),
        }
    _A_in = _A_setup()

    def _B_setup():
        B, Sq, D = 32, 48, 512
        Hq, Hkv, Sk, Dh = 32, 32, 48, 128
        assert Hq % Hkv == 0, (Hq, Hkv)
        return {
            "x": _w((lambda *s: _rng.normal(s) * 0.8)(B, Sq, D)),
            "k_cache": _w((lambda *s: _rng.normal(s) * 0.8)(B, Hkv, Sk, Dh)),
            "v_cache": _w((lambda *s: _rng.normal(s) * 0.05)(B, Hkv, Sk, Dh)),
            "wq": _w((lambda *s: _rng.normal(s) * 0.8)(D, Hq * Dh) * (D ** -0.5)),
            "wo": _w((lambda *s: _rng.normal(s) * 0.05)(Hq * Dh, D) * ((Hq * Dh) ** -0.5)),
        }
    _B_in = _B_setup()

    return {
        "A_x": _A_in["x"],
        "A_k_cache": _A_in["k_cache"],
        "A_v_cache": _A_in["v_cache"],
        "A_wq": _A_in["wq"],
        "A_wo": _A_in["wo"],
        "B_x": _B_in["x"],
        "B_k_cache": _B_in["k_cache"],
        "B_v_cache": _B_in["v_cache"],
        "B_wq": _B_in["wq"],
        "B_wo": _B_in["wo"],
    }

def reference(A_x, A_k_cache, A_v_cache, A_wq, A_wo, B_x, B_k_cache, B_v_cache, B_wq, B_wo):
    def _A_ref(x, k_cache, v_cache, wq, wo):
        B, Sq, D = x.shape
        Hq, Dh = 32, 128
        Hkv = k_cache.shape[1]
        rep = Hq // Hkv
        q = (lambda x, *d: x.transpose(*d))((x @ wq).reshape(B, Sq, Hq, Dh), 0, 2, 1, 3)
        k = jnp.repeat(k_cache, rep, axis=1)
        v = jnp.repeat(v_cache, rep, axis=1)
        scores = jnp.einsum("bhqd,bhkd->bhqk", q, k) * (Dh ** -0.5)
        p = _softmax(scores, axis=-1)
        o = jnp.einsum("bhqk,bhkd->bhqd", p, v)
        return (lambda x, *d: x.transpose(*d))(o, 0, 2, 1, 3).reshape(B, Sq, Hq * Dh) @ wo

    def _B_ref(x, k_cache, v_cache, wq, wo):
        B, Sq, D = x.shape
        Hq, Dh = 32, 128
        Hkv = k_cache.shape[1]
        rep = Hq // Hkv
        q = (lambda x, *d: x.transpose(*d))((x @ wq).reshape(B, Sq, Hq, Dh), 0, 2, 1, 3)
        k = jnp.repeat(k_cache, rep, axis=1)
        v = jnp.repeat(v_cache, rep, axis=1)
        scores = jnp.einsum("bhqd,bhkd->bhqk", q, k) * (Dh ** -0.5)
        p = _softmax(scores, axis=-1)
        o = jnp.einsum("bhqk,bhkd->bhqd", p, v)
        return (lambda x, *d: x.transpose(*d))(o, 0, 2, 1, 3).reshape(B, Sq, Hq * Dh) @ wo

    a = _A_ref(A_x, A_k_cache, A_v_cache, A_wq, A_wo)
    b = _B_ref(B_x, B_k_cache, B_v_cache, B_wq, B_wo)
    return jnp.concatenate([a, b], axis=-1)
```

```python
import math
import jax
import jax.numpy as jnp
from jax import lax
import jax.experimental.pallas as pl
import jax.experimental.pallas.tpu as pltpu

B, SQ, D = 32, 48, 512
H, SK, DH = 32, 48, 128
M_ALL = B * SQ
F32 = jnp.float32
BF16 = jnp.bfloat16


def make(bt=8, hg=4, skew=1, nobc=1, qf32=0):
    NC = B // bt
    NG = H // hg
    NSTEP = 2 * NG
    MC = bt * SQ
    GW = hg * DH
    NP = D // DH
    c_exp = float(DH ** -0.5) * math.log2(math.e)
    QDT = F32 if qf32 else BF16

    NRING = 4
    SEM_RING = 0
    SEM_P = NRING
    NPG = 7
    SEM_XB = SEM_P
    SEM_O = SEM_P + 1
    NSEM = SEM_P + NPG

    def kernel(ax, ak, av, awq, awo, bx, bk, bv, bwq, bwo, o_hbm,
               x_buf, wq_buf, wo_buf, k_buf, v_buf, q_buf, acc, stage, sems):
        src = ((ax, ak, av, awq, awo), (bx, bk, bv, bwq, bwo))

        def mult(v, m):
            return v if isinstance(v, int) else pl.multiple_of(v, m)

        def ring(s):
            return sems.at[SEM_RING + (s % NRING if isinstance(s, int) else jnp.bitwise_and(s, NRING - 1))]

        def cp_wq(brs, s, sem):
            g = s - brs * NG
            return pltpu.make_async_copy(src[brs][3].at[:, pl.ds(mult(g * GW, GW), GW)], wq_buf.at[s], sem)
        def cp_wo(brs, s, sem):
            g = s - brs * NG
            return pltpu.make_async_copy(src[brs][4].at[pl.ds(mult(g * GW, GW), GW), :], wo_buf.at[s], sem)
        def cp_k(brs, s, sem):
            g = s - brs * NG
            return pltpu.make_async_copy(src[brs][1].at[:, pl.ds(g * hg, hg)], k_buf.at[s], sem)
        def cp_v(brs, s, sem):
            g = s - brs * NG
            return pltpu.make_async_copy(src[brs][2].at[:, pl.ds(g * hg, hg)], v_buf.at[s], sem)
        def wait_buf(buf, sem):
            pltpu.make_async_copy(buf, buf, sem).wait()
        def psem(i):
            return sems.at[SEM_P + i]
        def cp_x(c0, c1, sem):
            r = pl.ds(c0 * MC, (c1 - c0) * MC)
            return pltpu.make_async_copy(ax.at[r], x_buf.at[0, r], sem)
        def cp_wq0(j0, j1, sem):
            cs = pl.ds(j0 * DH, (j1 - j0) * DH)
            return pltpu.make_async_copy(awq.at[:, cs], wq_buf.at[0, :, cs], sem)
        def cp_k0(c0, c1, sem):
            r = pl.ds(c0 * bt, (c1 - c0) * bt)
            return pltpu.make_async_copy(ak.at[r, pl.ds(0, hg)], k_buf.at[0, r], sem)
        def cp_v0(c0, c1, sem):
            r = pl.ds(c0 * bt, (c1 - c0) * bt)
            return pltpu.make_async_copy(av.at[r, pl.ds(0, hg)], v_buf.at[0, r], sem)
        cp_xb = pltpu.make_async_copy(bx, x_buf.at[1], sems.at[SEM_XB])
        cp_oa = pltpu.make_async_copy(stage.at[0], o_hbm.at[:, pl.ds(0, D)], sems.at[SEM_O])
        def cp_ob(c, n0, n1):
            r = pl.ds(c * MC, MC)
            return pltpu.make_async_copy(stage.at[1, r, pl.ds(n0 * DH, (n1 - n0) * DH)],
                                         o_hbm.at[r, pl.ds(D + n0 * DH, (n1 - n0) * DH)], sems.at[SEM_O])

        def qproj(s, c, j):
            br = s // NG
            x = x_buf[br, pl.ds(c * MC, MC), :]
            w = wq_buf[s, :, pl.ds(j * DH, DH)]
            q_buf[j, pl.ds(c * MC, MC), :] = jnp.dot(x, w, preferred_element_type=F32).astype(QDT)

        def step(s, do_q, hooks=None):
            hooks = hooks or {}
            br = s // NG
            g = s % NG
            first = g == 0
            st = {}
            o = {}
            ocat = {}

            def qk(c, j):
                res = []
                for b in range(bt):
                    qb = q_buf[j, pl.ds(c * MC + b * SQ, SQ), :].astype(BF16)
                    kb = k_buf[s, c * bt + b, j]
                    sc = lax.dot_general(qb, kb, (((1,), (1,)), ((), ())), preferred_element_type=F32)
                    m = jnp.max(sc, axis=-1, keepdims=True)
                    p = jnp.exp2((sc - m) * c_exp)
                    l = jnp.sum(p, axis=-1, keepdims=True)
                    res.append((p, pl.reciprocal(l, approx=True)))
                st[(c, j)] = res

            def pv(c, j):
                outs = []
                for b in range(bt):
                    p, inv = st[(c, j)][b]
                    vb = v_buf[s, c * bt + b, j]
                    ob = jnp.dot(p.astype(BF16), vb, preferred_element_type=F32)
                    outs.append(ob * inv)
                o[(c, j)] = jnp.concatenate(outs, axis=0)

            def oproj(c, n):
                if c not in ocat:
                    ocat[c] = jnp.concatenate([o[(c, j)] for j in range(hg)], axis=1).astype(BF16)
                w = wo_buf[s, :, pl.ds(n * DH, DH)]
                part = jnp.dot(ocat[c], w, preferred_element_type=F32)
                rows, cols = pl.ds(c * MC, MC), pl.ds(n * DH, DH)
                if isinstance(s, int):
                    new = part if first else acc[rows, cols] + part
                    if g != NG - 1:
                        acc[rows, cols] = new
                    else:
                        stage[br, rows, cols] = new.astype(BF16)
                else:
                    new = jnp.where(first, 0.0, acc[rows, cols]) + part
                    acc[rows, cols] = new
                    stage[br, rows, cols] = new.astype(BF16)

            subs = [(c, j) for c in range(NC) for j in range(hg)]
            oq = [(c, n) for c in range(NC) for n in range(NP)]
            done_pv = set()
            def o_ready(c):
                return all((c, j) in done_pv for j in range(hg))
            def run_o():
                c, n = oq.pop(0)
                oproj(c, n)
                if ('o_done', c, n) in hooks: hooks[('o_done', c, n)]()
            n_sub = len(subs)
            for i in range(n_sub + skew):
                if i < n_sub:
                    if ('qk',) + subs[i] in hooks: hooks[('qk',) + subs[i]]()
                    qk(*subs[i])
                    if do_q:
                        qproj(s + 1, *subs[i])
                if oq and o_ready(oq[0][0]) and i < n_sub - 1 + skew:
                    run_o()
                if i - skew >= 0:
                    pv(*subs[i - skew])
                    done_pv.add(subs[i - skew])
            while oq:
                run_o()

        hh = hg // 2
        groups = [
            [cp_x(0, 1, psem(0)), cp_wq0(0, hh, psem(0))],
            [cp_wq0(hh, hg, psem(1))],
            [cp_x(1, 2, psem(2))],
            [cp_x(2, NC, psem(3))],
            [cp_k0(0, 1, psem(4)), cp_v0(0, 1, psem(4)), cp_wq(0, 1, psem(4))],
            [cp_wo(0, 0, psem(5)), cp_k0(1, 2, psem(5)), cp_v0(1, 2, psem(5))],
            [cp_k0(2, NC, psem(6)), cp_v0(2, NC, psem(6))],
        ]
        for grp in groups:
            for cp in grp:
                cp.start()
        for t in (1, 2):
            cp_k(0, t, ring(t)).start(); cp_v(0, t, ring(t)).start(); cp_wo(0, t, ring(t)).start(); cp_wq(0, t + 1, ring(t)).start()
        def gwait(i):
            for cp in groups[i]:
                cp.wait()

        gwait(0)
        for j in range(hh):
            qproj(0, 0, j)
        gwait(1)
        for j in range(hh, hg):
            qproj(0, 0, j)
        gwait(2)
        for j in range(hg):
            qproj(0, 1, j)
        gwait(3)
        for c in range(2, NC):
            for j in range(hg):
                qproj(0, c, j)
        gwait(4)
        step(0, True, hooks={('qk', 1, 0): lambda: gwait(5), ('qk', 2, 0): lambda: gwait(6)})
        cp_xb.start()

        def issue(t):
            sem = ring(t)
            @pl.when(t < NG)
            def _():
                cp_k(0, t, sem).start(); cp_v(0, t, sem).start(); cp_wo(0, t, sem).start()
            @pl.when(jnp.logical_and(t >= NG, t < NSTEP))
            def _():
                cp_k(1, t, sem).start(); cp_v(1, t, sem).start(); cp_wo(1, t, sem).start()
            @pl.when(t + 1 < NG)
            def _():
                cp_wq(0, t + 1, sem).start()
            @pl.when(jnp.logical_and(t + 1 >= NG, t + 1 < NSTEP))
            def _():
                cp_wq(1, t + 1, sem).start()

        def body(s, carry):
            sem = ring(s)
            wait_buf(k_buf.at[s], sem)
            wait_buf(v_buf.at[s], sem)
            wait_buf(wo_buf.at[s], sem)
            wait_buf(wq_buf.at[s + 1], sem)
            @pl.when(s == NG - 1)
            def _():
                cp_xb.wait()
            @pl.when(s == NG)
            def _():
                cp_oa.start()
            step(s, True)
            issue(s + 2)
            return carry
        lax.fori_loop(1, NSTEP - 1, body, 0)

        s = NSTEP - 1
        sem = ring(s)
        wait_buf(k_buf.at[s], sem)
        wait_buf(v_buf.at[s], sem)
        wait_buf(wo_buf.at[s], sem)
        outs = {('o_done', c, NP - 1): cp_ob(c, 0, NP) for c in range(NC - 1)}
        outs.update({('o_done', NC - 1, n): cp_ob(NC - 1, n, n + 1) for n in range(NP)})
        step(s, False, hooks={k: cp.start for k, cp in outs.items()})
        cp_oa.wait()
        for cp in outs.values():
            cp.wait()

    def fn(A_x, A_k_cache, A_v_cache, A_wq, A_wo, B_x, B_k_cache, B_v_cache, B_wq, B_wo):
        anyspec = pl.BlockSpec(memory_space=pl.ANY)
        out = pl.pallas_call(
            kernel,
            in_specs=[anyspec] * 10,
            out_specs=anyspec,
            out_shape=jax.ShapeDtypeStruct((M_ALL, 2 * D), BF16),
            scratch_shapes=[
                pltpu.VMEM((2, M_ALL, D), BF16),
                pltpu.VMEM((NSTEP, D, GW), BF16),
                pltpu.VMEM((NSTEP, GW, D), BF16),
                pltpu.VMEM((NSTEP, B, hg, SK, DH), BF16),
                pltpu.VMEM((NSTEP, B, hg, SK, DH), BF16),
                pltpu.VMEM((hg, M_ALL, DH), QDT),
                pltpu.VMEM((M_ALL, D), F32),
                pltpu.VMEM((2, M_ALL, D), BF16),
                pltpu.SemaphoreType.DMA((NSEM,)),
            ],
            compiler_params=pltpu.CompilerParams(vmem_limit_bytes=110 * 1024 * 1024, disable_bounds_checks=bool(nobc)),
        )(A_x.reshape(M_ALL, D), A_k_cache, A_v_cache, A_wq, A_wo,
          B_x.reshape(M_ALL, D), B_k_cache, B_v_cache, B_wq, B_wo)
        return out.reshape(B, SQ, 2 * D)
    return fn

_impl = make()


@jax.jit
def pallas_concat_heads__gqa_block_cached__gqa_block_cached__near_ridge_kernel(
    A_x, A_k_cache, A_v_cache, A_wq, A_wo, B_x, B_k_cache, B_v_cache, B_wq, B_wo,
):
    return _impl(A_x, A_k_cache, A_v_cache, A_wq, A_wo, B_x, B_k_cache, B_v_cache, B_wq, B_wo)
```

```python
import math
import contextlib
import jax
import jax.numpy as jnp
from jax import lax
import jax.experimental.pallas as pl
import jax.experimental.pallas.tpu as pltpu

B, SQ, D = 32, 48, 512
H, SK, DH = 32, 48, 128
M_ALL = B * SQ
F32 = jnp.float32
BF16 = jnp.bfloat16
U32 = jnp.uint32

L_TERMS = {1: ((0, 0, 1), (1, 1, 1)), 2: ((1, 0, 1), (1, 1, 1)), 3: ((0, 0, 1),), 4: ((1, 1, 1),),
           5: ((0, 0, 1), (0, 1, 1)), 6: ((1, 0, 1), (0, 0, -1)), 7: ((0, 1, 1), (1, 1, -1))}
R_TERMS = {1: ((0, 0, 1), (1, 1, 1)), 2: ((0, 0, 1),), 3: ((0, 1, 1), (1, 1, -1)), 4: ((1, 0, 1), (0, 0, -1)),
           5: ((1, 1, 1),), 6: ((0, 0, 1), (0, 1, 1)), 7: ((1, 0, 1), (1, 1, 1))}
C_TERMS = {(0, 0): ((1, 1), (4, 1), (5, -1), (7, 1)), (0, 1): ((3, 1), (5, 1)),
           (1, 0): ((2, 1), (4, 1)), (1, 1): ((1, 1), (2, -1), (3, 1), (6, 1))}
SWAP = {1: 0, 7: 1, 6: 1, 4: 0, 5: 1, 2: 1, 3: 0}
O_OUTER = (2, 4, 5, 1, 7, 3, 6)
O_INNER = (3, 5, 2, 4, 1, 7, 6)
_STRAY = [(3, 1), (3, 7), (3, 6), (6, 1), (6, 7)]
ROUNDS = []
for _n, _i in enumerate(O_OUTER[:5]):
    ROUNDS.append([(_i, _j) for _j in (3, 5, 2, 4)])
    ROUNDS.append([(_i, _j) for _j in (1, 7, 6)] + [_STRAY[_n]])
ROUNDS += [[(3, _j) for _j in (3, 5, 2, 4)], [(6, _j) for _j in (3, 5, 2, 4)], [(6, 6)]]
FIRST_USE = {i: min(n for n, r in enumerate(ROUNDS) if any(p[0] == i for p in r)) for i in O_OUTER}
LAST_USE = {i: max(n for n, r in enumerate(ROUNDS) if any(p[0] == i for p in r)) for i in O_OUTER}
UPDATES = []
_seen = set()
for _r in ROUNDS:
    _u = []
    for _i in dict.fromkeys(p[0] for p in _r):
        for _blk, _terms in C_TERMS.items():
            _t = [(j, sg) for (j, sg) in _terms if (_i, j) in _r]
            if _t:
                _t.sort(key=lambda e: -e[1])
                _u.append((_i, _blk, _t, (_i, _blk) not in _seen))
                _seen.add((_i, _blk))
    UPDATES.append(_u)


def comb(terms, blk):
    if len(terms) == 1:
        return blk(terms[0][0], terms[0][1])
    (r0, c0, _), (r1, c1, sg) = terms
    a, b = blk(r0, c0), blk(r1, c1)
    return a + b if sg > 0 else a - b


def lin(terms, get):
    val = get(terms[0][0])
    for k, sg in terms[1:]:
        val = val + get(k) if sg > 0 else val - get(k)
    return val


def lazy(fn):
    cache = {}
    def get(*k):
        if k not in cache:
            cache[k] = fn(*k)
        return cache[k]
    return get


def make(nobc=1, lat_sm=330, lat_o=200, verbose=0, scopes=0, sdelay=1, finloop=1, fslab=16, epace=800, nosc=1, opfirst=1, fpos='q2', exact=1, tail=1, pvlate=1):
    hg = 4
    NU = 4
    bt = 4 * NU
    NC = B // bt
    NG = H // hg
    NSTEP = 2 * NG
    MU = 4 * SQ
    MC = bt * SQ
    MQ = NU * SQ
    GW = hg * DH
    XC = 384
    QR = 192
    NGRP = B // 2
    c_exp = float(DH ** -0.5) * math.log2(math.e)

    NRING = 4
    SEM_RING = 0
    SEM_P = NRING
    NPG = 7
    SEM_XB = SEM_P
    SEM_O = SEM_P + 1
    NSEM = SEM_P + NPG

    def scope(name):
        return jax.named_scope(name) if scopes else contextlib.nullcontext()

    def dot(a, b):
        return jnp.dot(a, b, preferred_element_type=F32)

    def kernel(ax, ak, av, awq, awo, bx, bk, bv, bwq, bwo, o_hbm,
               x_buf, wq_buf, wo_buf, k_buf, v_buf, q_buf, od_buf, s_buf, ro_buf, accm, cb_buf, stage, sems):
        src = ((ax, ak, av, awq, awo), (bx, bk, bv, bwq, bwo))

        def mult(v, m):
            return v if isinstance(v, int) else pl.multiple_of(v, m)

        def slot(s):
            return s % NRING if isinstance(s, int) else jnp.bitwise_and(s, NRING - 1)

        def ring(s):
            return sems.at[SEM_RING + slot(s)]

        def cp_wq(brs, s, sem):
            g = s - brs * NG
            return pltpu.make_async_copy(src[brs][3].at[:, pl.ds(mult(g * GW, GW), GW)], wq_buf.at[slot(s)], sem)
        def cp_wo(brs, s, sem):
            g = s - brs * NG
            return pltpu.make_async_copy(src[brs][4].at[pl.ds(mult(g * GW, GW), GW), :], wo_buf.at[slot(s)], sem)
        def cp_k(brs, s, sem):
            g = s - brs * NG
            return pltpu.make_async_copy(src[brs][1].at[:, pl.ds(g * hg, hg)], k_buf.at[slot(s)], sem)
        def cp_v(brs, s, sem):
            g = s - brs * NG
            return pltpu.make_async_copy(src[brs][2].at[:, pl.ds(g * hg, hg)], v_buf.at[slot(s)], sem)
        def wait_buf(buf, sem):
            pltpu.make_async_copy(buf, buf, sem).wait()
        def psem(i):
            return sems.at[SEM_P + i]
        def cp_x(c0, c1, sem):
            r = pl.ds(c0 * XC, (c1 - c0) * XC)
            return pltpu.make_async_copy(ax.at[r], x_buf.at[0, r], sem)
        def cp_wq0(j0, j1, sem):
            cs = pl.ds(j0 * DH, (j1 - j0) * DH)
            return pltpu.make_async_copy(awq.at[:, cs], wq_buf.at[0, :, cs], sem)
        def cp_k0(c0, c1, sem):
            r = pl.ds(c0 * 8, (c1 - c0) * 8)
            return pltpu.make_async_copy(ak.at[r, pl.ds(0, hg)], k_buf.at[0, r], sem)
        def cp_v0(c0, c1, sem):
            r = pl.ds(c0 * 8, (c1 - c0) * 8)
            return pltpu.make_async_copy(av.at[r, pl.ds(0, hg)], v_buf.at[0, r], sem)
        cp_xb = pltpu.make_async_copy(bx, x_buf.at[1], sems.at[SEM_XB])
        def cp_o(br, r0, nr, c0, ncol):
            r = pl.ds(r0, nr)
            return pltpu.make_async_copy(stage.at[br, r, pl.ds(c0, ncol)],
                                         o_hbm.at[r, pl.ds(br * D + c0, ncol)], sems.at[SEM_O])

        def unpk(w, idx):
            return pltpu.unpack_elementwise(w, index=idx, packed_dtype=BF16, unpacked_dtype=F32)
        def pk(lo, hi):
            return pltpu.pack_elementwise([lo, hi], packed_dtype=BF16)

        def ro_pieces(s):
            def piece(i, r0):
                def srcw(r1, c1, r2, c2):
                    v = wo_buf[slot(s), pl.ds((2 * r1 + r2) * DH + r0, 16), pl.ds((2 * c1 + (c2 ^ SWAP[i])) * DH, DH)]
                    return pltpu.bitcast(v, U32)
                srcw = lazy(srcw)
                half = [lazy(lambda r2, c2, h=h: comb(R_TERMS[i], lambda r1, c1: unpk(srcw(r1, c1, r2, c2), h))) for h in range(2)]
                for j in range(1, 8):
                    if len(R_TERMS[i]) == 1 and len(R_TERMS[j]) == 1:
                        val = srcw(R_TERMS[i][0][0], R_TERMS[i][0][1], R_TERMS[j][0][0], R_TERMS[j][0][1])
                    else:
                        val = pk(comb(R_TERMS[j], half[0]), comb(R_TERMS[j], half[1]))
                    ro_buf[i - 1, j - 1, pl.ds(r0 // 2, 8), :] = val
            return [lambda i=i, r0=r0: piece(i, r0) for i in O_OUTER for r0 in range(0, DH, 16)]

        def fin_piece(br, su, r0):
            c, u = (su // NU, su % NU) if isinstance(su, int) else (lax.shift_right_logical(su, 2), jnp.bitwise_and(su, NU - 1))
            rows = pl.ds(mult(u * SQ + r0, 8), 8)
            inner = lazy(lambda k, r2, c2: accm[br, c, k - 1, 2 * r2 + c2, rows, :])
            for (r1, c1) in C_TERMS:
                for r2 in range(2):
                    val = jnp.concatenate([lin(C_TERMS[(r1, c1)], lambda k: inner(k, r2, c2)) for c2 in range(2)], axis=1)
                    stage[br, pl.ds(mult(su * MU + (2 * r1 + r2) * SQ + r0, 8), 8), pl.ds(c1 * 2 * DH, 2 * DH)] = val.astype(BF16)
        def fin_pieces(br, su):
            return [lambda r0=r0: fin_piece(br, su, r0) for r0 in range(0, SQ, 8)]

        def inc_fin(br, c, i):
            for r0 in range(0, MQ, fslab):
                rows = pl.ds(r0, fslab)
                for r2 in range(2):
                    n = jnp.concatenate([accm[br, c, i - 1, 2 * r2 + c2, rows, :] for c2 in range(2)], axis=1)
                    for (r1, c1), terms in C_TERMS.items():
                        order = [k for k in O_OUTER if k in dict(terms)]
                        if i not in order:
                            continue
                        sg = dict(terms)[i]
                        idx = (2 * r1 + c1, r2, rows, slice(None))
                        if i == order[0]:
                            val = n if sg > 0 else -n
                        else:
                            val = cb_buf[idx] + n if sg > 0 else cb_buf[idx] - n
                        if i == order[-1]:
                            u, r = r0 // SQ, r0 % SQ
                            stage[br, pl.ds(c * MC + u * MU + (2 * r1 + r2) * SQ + r, fslab), pl.ds(c1 * 2 * DH, 2 * DH)] = val.astype(BF16)
                        else:
                            cb_buf[idx] = val

        def qproj(s, r0, nr, j):
            br = s // NG
            x = x_buf[br, pl.ds(r0, nr), :]
            w = wq_buf[slot(s), :, pl.ds(j * DH, DH)]
            q_buf[j, pl.ds(r0, nr), :] = dot(x, w).astype(BF16)

        def emit(tasks, fills=()):
            fillers = {}
            for pieces, lo, hi in fills:
                n = len(pieces)
                for k, p in enumerate(pieces):
                    pos = lo + (k * (hi - lo)) // n
                    fillers.setdefault(pos, []).append(p)
            for idx, run in enumerate(tasks):
                run()
                for p in fillers.get(idx, []): p()

        lane = lax.broadcasted_iota(jnp.int32, (SK, 2 * SQ), 1)

        def slab_reduce(x, op, red):
            acc = x[0:8]
            for r in range(8, x.shape[0], 8):
                acc = op(acc, x[r:r + 8])
            return red(acc, axis=0, keepdims=True)

        def step(s, do_q, hooks=None, fills=None, prev=True, defer=True, ro_at='k4'):
            hooks = hooks or {}
            br = s // NG
            sl = slot(s)
            static = isinstance(s, int)
            pt, mx = {}, {}

            def qkr(g):
                if ('qk', g) in hooks: hooks[('qk', g)]()
                b0 = 2 * g
                for j in range(hg):
                    q2 = q_buf[j, pl.ds(b0 * SQ, 2 * SQ), :]
                    k2 = jnp.concatenate([k_buf[sl, b0 + r, j, pl.ds(r0, 16), :] for r0 in range(0, SK, 16) for r in range(2)], axis=0)
                    st = lax.dot_general(k2, q2, (((1,), (1,)), ((), ())), preferred_element_type=F32)
                    top = jnp.concatenate([st[r0:r0 + 16] for r0 in range(0, 2 * SK, 32)], axis=0)
                    bot = jnp.concatenate([st[r0 + 16:r0 + 32] for r0 in range(0, 2 * SK, 32)], axis=0)
                    sc = jnp.where(lane < SQ, top, bot)
                    mx[(g, j)] = slab_reduce(sc, jnp.maximum, jnp.max)
                    s_buf[g % 2, j] = sc

            def soft(g):
                for j in range(hg):
                    p = jnp.exp2((s_buf[g % 2, j] - mx[(g, j)]) * c_exp)
                    l = slab_reduce(p, jnp.add, jnp.sum)
                    p = p * pl.reciprocal(l, approx=not exact)
                    pt[(g, j)] = p.astype(BF16).T

            def pvr(g):
                c, u, bp = g // (2 * NU), (g // 2) % NU, g % 2
                for r in range(2):
                    for j in range(hg):
                        od_buf[c, 2 * bp + r, j, pl.ds(u * SQ, SQ), :] = dot(pt[(g, j)][r * SQ:(r + 1) * SQ], v_buf[sl, 2 * g + r, j])

            def oround(c, n, is_prev):
                sa = s - 1 if is_prev else s
                abr = sa // NG
                init = sa % NG == 0
                def rows(part):
                    return slice(None) if part is None else pl.ds(part * (MQ // 4), MQ // 4)
                raw = lazy(lambda rq, j, part: od_buf[c, rq, j, rows(part), :])
                inner = lazy(lambda i, r2, c2, part: comb(L_TERMS[i], lambda r1, c1: raw(2 * r1 + r2, 2 * c1 + c2, part)))
                parts = [None] if len(ROUNDS[n]) == 4 else range(4)
                res = {}
                for part in parts:
                    for i, j in ROUNDS[n]:
                        lhs = comb(L_TERMS[j], lambda r2, c2: inner(i, r2, c2, part)).astype(BF16)
                        res[(i, j, part)] = dot(lhs, pltpu.bitcast(ro_buf[i - 1, j - 1], BF16))
                for part in parts:
                    for i, (r2, c2), terms, first_touch in UPDATES[n]:
                        val = lin(terms, lambda j: res[(i, j, part)])
                        idx = (abr, c, i - 1, 2 * r2 + (c2 ^ SWAP[i]), rows(part), slice(None))
                        if not first_touch:
                            accm[idx] = accm[idx] + val
                        elif static:
                            accm[idx] = val if init else accm[idx] + val
                        else:
                            accm[idx] = jnp.where(init, 0.0, accm[idx]) + val
                if not is_prev and ('or', c, n) in hooks: hooks[('or', c, n)]()

            qks = list(range(NGRP))
            pvs = list(range(NGRP))
            qq = [(r0, j) for r0 in range(0, M_ALL, QR) for j in range(hg)] if do_q else []
            oq = [(-1, n) for n in range(13)] if prev else []
            oq += [(c, n) for c in range(NC - 1 if defer else NC) for n in range(13)]
            t = 0
            qk_end, pv_end = {}, {}
            log, tasks = [], []
            total = 96 * 2 * NGRP + QR * len(qq) + sum(MQ if n < 12 else MQ // 4 for _, n in oq)
            def add_qk():
                nonlocal t
                g = qks.pop(0)
                tasks.append(lambda: qkr(g)); t += 96; qk_end[g] = t; log.append('k%d' % g)
            def pv_ready():
                return bool(pvs) and pvs[0] in qk_end and qk_end[pvs[0]] + lat_sm <= t
            def add_pv():
                nonlocal t
                g = pvs.pop(0)
                tasks.append(lambda: pvr(g)); t += 96; pv_end[g] = t; log.append('PV%d' % g)
            def o_ready():
                if not oq: return False
                c = oq[0][0]
                g = (c + 1) * 2 * NU - 1
                return c < 0 or (g in pv_end and pv_end[g] + lat_o <= t)
            def q_ready():
                return bool(qq) and (qq[0][0] + QR) // (2 * SQ) - 1 in qk_end
            def add_o():
                nonlocal t
                c, n = oq.pop(0)
                tasks.append(lambda: oround(NC - 1 if c < 0 else c, n, c < 0)); log.append(('Op' if c < 0 else f'O{c}') + f'_{n}')
                t += MQ if n < 12 else MQ // 4
            def add_q():
                nonlocal t
                r0, j = qq.pop(0)
                tasks.append(lambda: qproj(s + 1, r0, QR, j)); t += QR
                log.append(f'Q{r0 // QR}_{j}')
            def pv_ok():
                return not (pvs[0] >= (NC - 1) * 2 * NU and oq and oq[0][0] < 0)
            if do_q:
                n_o = len(oq)
                if opfirst and prev: add_o()
                add_qk()
                for g in range(1, NGRP):
                    add_qk()
                    while q_ready() and not pv_ready():
                        add_q()
                    tgt = n_o - (n_o * g) // (NGRP - 1)
                    if pvlate:
                        while pvs and pvs[0] < g:
                            add_pv()
                        while len(oq) > tgt and o_ready():
                            add_o()
                    while pvs and pvs[0] <= g:
                        while not pv_ok(): add_o()
                        t = max(t, qk_end[pvs[0]] + lat_sm)
                        add_pv()
                    while len(oq) > tgt and o_ready():
                        add_o()
                while qq or oq:
                    if o_ready(): add_o()
                    elif qq: add_q()
                    else: t += 8
            pace = (total - 13 * MQ - epace) // NGRP
            while qks or pvs or oq or qq:
                if pv_ready() and pv_ok():
                    add_pv(); continue
                if qks and t >= (NGRP - len(qks)) * pace and len(pvs) - len(qks) < 2:
                    add_qk(); continue
                if o_ready():
                    add_o(); continue
                if qks and len(pvs) - len(qks) < 2:
                    add_qk(); continue
                t += 8
            if verbose:
                print(' '.join(log), 't=', t, 'total', total)
            fl = []
            for g in range(NGRP):
                p = log.index('k%d' % g)
                lim = log.index('PV%d' % g) - 1
                if g + 2 < NGRP: lim = min(lim, log.index('k%d' % (g + 2)) - 1)
                p = min(p + sdelay, lim)
                fl.append(([lambda g=g: soft(g)], p, p + 1))
            rp = ro_pieces(s)
            for n, i in enumerate(O_OUTER):
                last_use, first_use = LAST_USE[i], FIRST_USE[i]
                lo = log.index(f'Op_{last_use}') if prev else log.index(ro_at)
                hi = log.index(f'O0_{first_use}')
                fl.append((rp[8 * n:8 * n + 8], lo, max(lo + 1, hi - 1)))
            emit(tasks, fl + (fills(log) if fills else []))

        hh = hg // 2
        groups = [
            [cp_x(0, 1, psem(0)), cp_wq0(0, hh, psem(0))],
            [cp_wq0(hh, hg, psem(1))],
            [cp_x(1, 2, psem(2))],
            [cp_x(2, 4, psem(3))],
            [cp_k0(0, 1, psem(4)), cp_v0(0, 1, psem(4)), cp_wq(0, 1, psem(4))],
            [cp_k0(1, 2, psem(5)), cp_v0(1, 2, psem(5))],
            [cp_wo(0, 0, psem(6)), cp_k0(2, 4, psem(6)), cp_v0(2, 4, psem(6))],
        ]
        for grp in groups:
            for cp in grp:
                cp.start()
        for t in (1, 2):
            cp_k(0, t, ring(t)).start(); cp_v(0, t, ring(t)).start(); cp_wo(0, t, ring(t)).start(); cp_wq(0, t + 1, ring(t)).start()
        def gwait(i):
            with scope(f'w{i}'):
                for cp in groups[i]:
                    cp.wait()

        gwait(0)
        for j in range(hh): qproj(0, 0, XC, j)
        gwait(1)
        for j in range(hh, hg): qproj(0, 0, XC, j)
        gwait(2)
        for j in range(hg): qproj(0, XC, XC, j)
        gwait(3)
        for c in (2, 3):
            for j in range(hg): qproj(0, c * XC, XC, j)
        gwait(4)
        step(0, True, prev=False, ro_at='k8', hooks={('qk', 4): lambda: gwait(5), ('qk', 8): lambda: gwait(6)})
        cp_xb.start()

        def issue(t):
            sem = ring(t)
            @pl.when(t < NG)
            def _():
                cp_k(0, t, sem).start(); cp_v(0, t, sem).start(); cp_wo(0, t, sem).start()
            @pl.when(jnp.logical_and(t >= NG, t < NSTEP))
            def _():
                cp_k(1, t, sem).start(); cp_v(1, t, sem).start(); cp_wo(1, t, sem).start()
            @pl.when(t + 1 < NG)
            def _():
                cp_wq(0, t + 1, sem).start()
            @pl.when(jnp.logical_and(t + 1 >= NG, t + 1 < NSTEP))
            def _():
                cp_wq(1, t + 1, sem).start()

        def body(s, carry):
            sem = ring(s)
            with scope('wait'):
                wait_buf(k_buf.at[slot(s)], sem)
                wait_buf(v_buf.at[slot(s)], sem)
                wait_buf(wo_buf.at[slot(s)], sem)
                wait_buf(wq_buf.at[slot(s + 1)], sem)
                @pl.when(s == NG - 1)
                def _():
                    cp_xb.wait()
            fills = None
            if finloop:
                su = jnp.maximum(s - NG, 0)
                fp = fin_pieces(0, su)
                def fills(log):
                    if fpos == 'q2':
                        pos = [log.index('k%d' % (10 + n)) + 1 for n in range(6)]
                    elif fpos == 'oo':
                        pos = [i for i in range(len(log) - 1) if log[i][0] == 'O' and log[i + 1][0] == 'O'][-6:]
                    elif fpos == 'oo1':
                        pos = [i for i in range(len(log) - 1) if log[i][0] == 'O' and log[i + 1][0] == 'O'][:6]
                    elif fpos == 'first':
                        pos = [log.index('k%d' % (2 + n)) + 1 for n in range(6)]
                    elif fpos == 'end':
                        pos = [len(log) - 3] * 6
                    return [([p], i, i + 1) for p, i in zip(fp, pos)]
            step(s, True, fills=fills)
            issue(s + 2)
            return carry
        lax.fori_loop(1, NSTEP - 1, body, 0)

        s = NSTEP - 1
        sem = ring(s)
        outs = []
        def start_out(*a):
            cp = cp_o(*a)
            outs.append(cp)
            cp.start()
        n_done = (NSTEP - 1 - NG) if finloop else 0
        if n_done:
            start_out(0, 0, n_done * MU, 0, D)
        with scope('wE'):
            wait_buf(k_buf.at[slot(s)], sem)
            wait_buf(v_buf.at[slot(s)], sem)
            wait_buf(wo_buf.at[slot(s)], sem)
        fin_a = []
        for su in range(n_done, NC * NU):
            fin_a += fin_pieces(0, su)
        fin_a.append(lambda: start_out(0, n_done * MU, M_ALL - n_done * MU, 0, D))
        hooks = {}
        def hook(c, n):
            for k, i in enumerate(O_OUTER):
                if LAST_USE[i] == n:
                    inc_fin(1, c, i)
                    for (r1, c1), terms in C_TERMS.items():
                        if [q for q in O_OUTER if q in dict(terms)][-1] == i and c == NC - 1:
                            for u in range(NU):
                                start_out(1, c * MC + u * MU + 2 * r1 * SQ, 2 * SQ, c1 * 2 * DH, 2 * DH)
            if n == 12 and c < NC - 1:
                start_out(1, c * MC, MC, 0, D)
        for c in range(NC):
            for n in range(13):
                hooks[('or', c, n)] = lambda c=c, n=n: hook(c, n)
        step(s, False, defer=False, hooks=hooks, fills=lambda log: [(fin_a, 1, 12)])
        with scope('wout'):
            for cp in outs:
                cp.wait()

    def fn(A_x, A_k_cache, A_v_cache, A_wq, A_wo, B_x, B_k_cache, B_v_cache, B_wq, B_wo):
        anyspec = pl.BlockSpec(memory_space=pl.ANY)
        out = pl.pallas_call(
            kernel,
            in_specs=[anyspec] * 10,
            out_specs=anyspec,
            out_shape=jax.ShapeDtypeStruct((M_ALL, 2 * D), BF16),
            scratch_shapes=[
                pltpu.VMEM((2, M_ALL, D), BF16),
                pltpu.VMEM((NRING, D, GW), BF16),
                pltpu.VMEM((NRING, GW, D), BF16),
                pltpu.VMEM((NRING, B, hg, SK, DH), BF16),
                pltpu.VMEM((NRING, B, hg, SK, DH), BF16),
                pltpu.VMEM((hg, M_ALL, DH), BF16),
                pltpu.VMEM((NC, 4, 4, MQ, DH), F32),
                pltpu.VMEM((2, 4, SK, 2 * SQ), F32),
                pltpu.VMEM((7, 7, DH // 2, DH), U32),
                pltpu.VMEM((2, NC, 7, 4, MQ, DH), F32),
                pltpu.VMEM((4, 2, MQ, 2 * DH), F32),
                pltpu.VMEM((2, M_ALL, D), BF16),
                pltpu.SemaphoreType.DMA((NSEM,)),
            ],
            compiler_params=pltpu.CompilerParams(vmem_limit_bytes=100 * 1024 * 1024, disable_bounds_checks=bool(nobc),
                                                 disable_semaphore_checks=bool(nosc)),
        )(A_x.reshape(M_ALL, D), A_k_cache, A_v_cache, A_wq, A_wo,
          B_x.reshape(M_ALL, D), B_k_cache, B_v_cache, B_wq, B_wo)
        return out.reshape(B, SQ, 2 * D)
    return fn

_impl = make(exact=0, opfirst=0, fpos='first')


@jax.jit
def pallas_concat_heads__gqa_block_cached__gqa_block_cached__near_ridge_kernel(
    A_x, A_k_cache, A_v_cache, A_wq, A_wo, B_x, B_k_cache, B_v_cache, B_wq, B_wo,
):
    return _impl(A_x, A_k_cache, A_v_cache, A_wq, A_wo, B_x, B_k_cache, B_v_cache, B_wq, B_wo)
```

```python
import math

import jax
import jax.numpy as jnp
from jax import lax
import jax.experimental.pallas as pl
import jax.experimental.pallas.tpu as pltpu

F32 = jnp.float32
BF16 = jnp.bfloat16

B, SQ, D = 32, 48, 512
H, SK, DH = 32, 48, 128
M_ALL = B * SQ
HG = 4
NG = H // HG
NSTEP = 2 * NG
GW = HG * DH
NPAIR = B // 2
NC = 2
MC = M_ALL // NC
MQ = MC // 4
QR = 192
XC = 384
C_EXP = float(DH ** -0.5) * math.log2(math.e)

NRING = 4
SEM_P = NRING
SEM_XB = SEM_P
SEM_O = SEM_P + 1
NSEM = SEM_P + 7

L_TERMS = {1: ((0, 0, 1), (1, 1, 1)), 2: ((1, 0, 1), (1, 1, 1)), 3: ((0, 0, 1),), 4: ((1, 1, 1),),
           5: ((0, 0, 1), (0, 1, 1)), 6: ((1, 0, 1), (0, 0, -1)), 7: ((0, 1, 1), (1, 1, -1))}
R_TERMS = {1: ((0, 0, 1), (1, 1, 1)), 2: ((0, 0, 1),), 3: ((0, 1, 1), (1, 1, -1)), 4: ((1, 0, 1), (0, 0, -1)),
           5: ((1, 1, 1),), 6: ((0, 0, 1), (0, 1, 1)), 7: ((1, 0, 1), (1, 1, 1))}
C_TERMS = {(0, 0): ((1, 1), (4, 1), (5, -1), (7, 1)), (0, 1): ((3, 1), (5, 1)),
           (1, 0): ((2, 1), (4, 1)), (1, 1): ((1, 1), (2, -1), (3, 1), (6, 1))}
SWAP = {1: 0, 2: 1, 3: 0, 4: 0, 5: 1, 6: 1, 7: 1}
OUTER = (2, 4, 3, 5, 1, 7, 6)

ROUNDS = []
for _i, _stray in zip(OUTER[:5], ((7, 1), (7, 7), (7, 6), (6, 1), (6, 7))):
    ROUNDS.append([(_i, _j) for _j in (3, 5, 2, 4)])
    ROUNDS.append([(_i, _j) for _j in (1, 7, 6)] + [_stray])
ROUNDS += [[(7, _j) for _j in (3, 5, 2, 4)], [(6, 6)], [(6, _j) for _j in (3, 5, 2, 4)]]
NR = len(ROUNDS)
FIRST_USE = {i: min(n for n, r in enumerate(ROUNDS) if any(p[0] == i for p in r)) for i in OUTER}
LAST_USE = {i: max(n for n, r in enumerate(ROUNDS) if any(p[0] == i for p in r)) for i in OUTER}
UPDATES = []
_seen = set()
for _r in ROUNDS:
    _u = []
    for _i in dict.fromkeys(p[0] for p in _r):
        for _blk, _terms in C_TERMS.items():
            _t = sorted(((j, sg) for (j, sg) in _terms if (_i, j) in _r), key=lambda e: -e[1])
            if _t:
                _u.append((_i, _blk, _t, (_i, _blk) not in _seen))
                _seen.add((_i, _blk))
    UPDATES.append(_u)

ORDER_FIRST = "kkqqpp" + "kqqp" * 7 + "kqqop" + "kqqoop" * 6 + "q"
ORDER_MID = "ckkqqpop" + "".join("kqq" + "o" * n + "p" for n in (2, 2, 1, 2, 2, 2, 1, 2, 2, 2, 1, 2, 2, 2)) + "q"
ORDER_LAST = "ckokopkopopkokopkopkopopkokopkoopkopkopkopopkokopkopop" + "o" * 22
N_HALVED = 5
FIN_AT = 6


def _comb(terms, blk):
    if len(terms) == 1:
        return blk(terms[0][0], terms[0][1])
    (r0, c0, _), (r1, c1, sg) = terms
    a, b = blk(r0, c0), blk(r1, c1)
    return a + b if sg > 0 else a - b


def _lin(terms, get):
    val = get(terms[0][0])
    for k, sg in terms[1:]:
        val = val + get(k) if sg > 0 else val - get(k)
    return val


def _lazy(fn):
    cache = {}

    def get(*k):
        if k not in cache:
            cache[k] = fn(*k)
        return cache[k]
    return get


def _dot(a, b):
    return jnp.dot(a, b, preferred_element_type=F32)


def _col_reduce(x, op, red):
    acc = x[0:8]
    for r in range(8, x.shape[0], 8):
        acc = op(acc, x[r:r + 8])
    return red(acc, axis=0, keepdims=True)


def _kernel(ax, ak, av, awq, awo, bx, bk, bv, bwq, bwo, o_hbm,
            x_buf, wq_buf, wo_buf, k_buf, v_buf, q_buf, o_buf, s_buf, r_buf, acc, c_buf, stage, sems):
    src = ((ax, ak, av, awq, awo), (bx, bk, bv, bwq, bwo))

    def slot(s):
        return s % NRING if isinstance(s, int) else jnp.bitwise_and(s, NRING - 1)

    def col0(g):
        return g * GW if isinstance(g, int) else pl.multiple_of(g * GW, GW)

    def cp_wq(br, s, sem):
        return pltpu.make_async_copy(src[br][3].at[:, pl.ds(col0(s - br * NG), GW)], wq_buf.at[slot(s)], sem)

    def cp_wo(br, s, sem):
        return pltpu.make_async_copy(src[br][4].at[pl.ds(col0(s - br * NG), GW), :], wo_buf.at[slot(s)], sem)

    def cp_kv(br, s, sem, b0=0, nb=B):
        heads, rows = pl.ds((s - br * NG) * HG, HG), pl.ds(b0, nb)
        return [pltpu.make_async_copy(src[br][1].at[rows, heads], k_buf.at[slot(s), rows], sem),
                pltpu.make_async_copy(src[br][2].at[rows, heads], v_buf.at[slot(s), rows], sem)]

    def cp_x(r0, nr, sem):
        return pltpu.make_async_copy(ax.at[pl.ds(r0, nr)], x_buf.at[0, pl.ds(r0, nr)], sem)

    def cp_wq0(c0, nc, sem):
        return pltpu.make_async_copy(awq.at[:, pl.ds(c0, nc)], wq_buf.at[0, :, pl.ds(c0, nc)], sem)

    cp_xb = pltpu.make_async_copy(bx, x_buf.at[1], sems.at[SEM_XB])

    def wait_step(s, with_wq=True):
        bufs = [k_buf.at[slot(s)], v_buf.at[slot(s)], wo_buf.at[slot(s)]]
        if with_wq:
            bufs.append(wq_buf.at[slot(s + 1)])
        for buf in bufs:
            pltpu.make_async_copy(buf, buf, sems.at[slot(s)]).wait()

    def qproj(s, r0, nr, j):
        x = x_buf[s // NG, pl.ds(r0, nr), :]
        w = wq_buf[slot(s), :, pl.ds(j * DH, DH)]
        q_buf[j, pl.ds(r0, nr), :] = _dot(x, w).astype(BF16)

    def wo_tile(s, i, r1, c1, r2, c2, r0=0, nr=DH):
        return wo_buf[slot(s), pl.ds((2 * r1 + r2) * DH + r0, nr), pl.ds((2 * c1 + (c2 ^ SWAP[i])) * DH, DH)]

    def plain(i, j):
        return len(R_TERMS[i]) == 1 and len(R_TERMS[j]) == 1

    def r_piece(s, i, r0):
        inner = _lazy(lambda r2, c2: _comb(R_TERMS[i], lambda r1, c1: wo_tile(s, i, r1, c1, r2, c2, r0, 16).astype(F32)))
        for j in range(1, 8):
            if not plain(i, j):
                r_buf[i - 1, j - 1, pl.ds(r0, 16), :] = _comb(R_TERMS[j], inner).astype(BF16)

    def fin_slab(br, p):
        c = (p >= MQ // 8).astype(jnp.int32)
        r0 = pl.multiple_of(p * 8 - c * MQ, 8)
        m = _lazy(lambda k, blk: acc[br, c, k - 1, blk, pl.ds(r0, 8), :])
        for (r1, c1), terms in C_TERMS.items():
            for r2 in range(2):
                val = jnp.concatenate([_lin(terms, lambda k: m(k, 2 * r2 + c2)) for c2 in range(2)], axis=1)
                row = pl.multiple_of(c * MC + (2 * r1 + r2) * MQ + r0, 8)
                stage[br, pl.ds(row, 8), pl.ds(c1 * 2 * DH, 2 * DH)] = val.astype(BF16)

    def fold(br, c, i, row0, nrows):
        for r0 in range(row0, row0 + nrows, 16):
            rows = pl.ds(r0, 16)
            for r2 in range(2):
                n = jnp.concatenate([acc[br, c, i - 1, 2 * r2 + c2, rows, :] for c2 in range(2)], axis=1)
                for (r1, c1), terms in C_TERMS.items():
                    order = [k for k in OUTER if k in dict(terms)]
                    if i not in order:
                        continue
                    pos = dict(terms)[i] > 0
                    idx = (2 * r1 + c1, r2, rows, slice(None))
                    if i == order[0]:
                        val = n if pos else -n
                    else:
                        val = c_buf[idx] + n if pos else c_buf[idx] - n
                    if i == order[-1]:
                        stage[br, pl.ds(c * MC + (2 * r1 + r2) * MQ + r0, 16), pl.ds(c1 * 2 * DH, 2 * DH)] = val.astype(BF16)
                    else:
                        c_buf[idx] = val

    lane = lax.broadcasted_iota(jnp.int32, (SK, DH), 1)

    def step(s, order, before_k=None, after_round=None, after_k=None):
        first, last = order is ORDER_FIRST, order is ORDER_LAST
        static = isinstance(s, int)
        sl = slot(s)
        pt, mx = {}, {}

        def scores(g):
            for j in range(HG):
                q2 = q_buf[j, pl.ds(2 * g * SQ, DH), :]
                k2 = jnp.concatenate([k_buf[sl, 2 * g + r, j, pl.ds(r0, 16), :]
                                      for r0 in range(0, SK, 16) for r in range(2)], axis=0)
                st = lax.dot_general(k2, q2, (((1,), (1,)), ((), ())), preferred_element_type=F32)
                top = jnp.concatenate([st[r0:r0 + 16] for r0 in range(0, 2 * SK, 32)], axis=0)
                bot = jnp.concatenate([st[r0 + 16:r0 + 32] for r0 in range(0, 2 * SK, 32)], axis=0)
                sc = jnp.where(lane < SQ, top, bot)
                mx[(g, j)] = _col_reduce(sc, jnp.maximum, jnp.max)
                s_buf[g % 2, j] = sc

        def softmax(g):
            for j in range(HG):
                p = jnp.exp2((s_buf[g % 2, j] - mx[(g, j)]) * C_EXP)
                p = p * pl.reciprocal(_col_reduce(p, jnp.add, jnp.sum), approx=True)
                pt[(g, j)] = p[:, :2 * SQ].astype(BF16).T

        def pv(g):
            c, blk, half = g // 8, (g // 2) % 4, g % 2
            for r in range(2):
                for j in range(HG):
                    o_buf[c, blk, j, pl.ds((2 * half + r) * SQ, SQ), :] = _dot(
                        pt[(g, j)][r * SQ:(r + 1) * SQ], v_buf[sl, 2 * g + r, j])

        def oround(sa, c, n, half):
            init = sa % NG == 0

            def rows(part):
                if half is not None:
                    return pl.ds(half * (MQ // 2), MQ // 2)
                return slice(None) if part is None else pl.ds(part * (MQ // 4), MQ // 4)

            raw = _lazy(lambda blk, j, part: o_buf[c, blk, j, rows(part), :])
            lin_ = _lazy(lambda i, r2, c2, part: _comb(L_TERMS[i], lambda r1, c1: raw(2 * r1 + r2, 2 * c1 + c2, part)))
            rin = _lazy(lambda i, r2, c2: _comb(R_TERMS[i], lambda r1, c1: wo_tile(sa, i, r1, c1, r2, c2).astype(F32)))
            parts = [None] if len(ROUNDS[n]) == 4 else range(4)
            res = {}
            for part in parts:
                for i, j in ROUNDS[n]:
                    lhs = _comb(L_TERMS[j], lambda r2, c2: lin_(i, r2, c2, part)).astype(BF16)
                    if plain(i, j):
                        rhs = wo_tile(sa, i, *R_TERMS[i][0][:2], *R_TERMS[j][0][:2])
                    elif first:
                        w = _comb(R_TERMS[j], lambda r2, c2: rin(i, r2, c2))
                        rhs = w.astype(BF16)
                        if part in (None, 0):
                            r_buf[i - 1, j - 1] = (w + 0.0).astype(BF16)
                    else:
                        rhs = r_buf[i - 1, j - 1]
                    res[(i, j, part)] = _dot(lhs, rhs)
            for part in parts:
                for i, (r2, c2), terms, first_touch in UPDATES[n]:
                    val = _lin(terms, lambda j: res[(i, j, part)])
                    idx = (sa // NG, c, i - 1, 2 * r2 + (c2 ^ SWAP[i]), rows(part), slice(None))
                    if not first_touch:
                        acc[idx] = acc[idx] + val
                    elif static:
                        acc[idx] = val if init else acc[idx] + val
                    else:
                        acc[idx] = jnp.where(init, 0.0, acc[idx]) + val

        qpieces = [(r0, j) for r0 in range(0, M_ALL, QR) for j in range(HG)]
        carried = qpieces.pop()
        rounds = [] if first else [(-1, n, None) for n in range(NR)]
        rounds += [(0, n, None) for n in range(NR)]
        if last:
            tail = range(NR - N_HALVED, NR)
            rounds += [(1, n, None) for n in range(NR) if n not in tail or len(ROUNDS[n]) != 4]
            rounds += [(1, n, h) for h in range(2) for n in tail if len(ROUNDS[n]) == 4]
        count = dict.fromkeys("kpqco", 0)
        tasks = []
        for t in order:
            n = count[t]
            count[t] += 1
            if t == "k":
                assert n - count["p"] < 2 and (first or count["c"] == 1)
                tasks.append(("k", n))
            elif t == "p":
                assert n < count["k"] and (first or n < 8 or count["o"] >= NR)
                tasks.append(("p", n))
            elif t == "q":
                assert qpieces[n][0] + QR <= count["k"] * 2 * SQ
                tasks.append(("q",) + qpieces[n])
            elif t == "c":
                tasks.append(("c",) + carried)
            else:
                assert count["p"] >= 8 * (rounds[n][0] + 1)
                tasks.append(("o",) + rounds[n])
        assert count["k"] == count["p"] == NPAIR and count["o"] == len(rounds)
        assert count["q"] == (0 if last else len(qpieces)) and count["c"] == (0 if first else 1)

        extra = {}
        for g in range(NPAIR):
            pos = min(tasks.index(("k", g)) + 1, tasks.index(("p", g)) - 1)
            extra.setdefault(pos, []).append(lambda g=g: softmax(g))
        if not first:
            for i in OUTER:
                lo = tasks.index(("o", -1, LAST_USE[i], None))
                hi = max(lo + 1, tasks.index(("o", 0, FIRST_USE[i], None)) - 1)
                for k in range(8):
                    extra.setdefault(lo + (k * (hi - lo)) // 8, []).append(lambda i=i, k=k: r_piece(s, i, 16 * k))
        for g, fn in (after_k or {}).items():
            extra.setdefault(tasks.index(("k", g)) + 1, []).append(fn)

        for pos, task in enumerate(tasks):
            if task[0] == "k":
                if before_k and task[1] in before_k:
                    before_k[task[1]]()
                scores(task[1])
            elif task[0] == "p":
                pv(task[1])
            elif task[0] == "q":
                qproj(s + 1, task[1], QR, task[2])
            elif task[0] == "c":
                qproj(s, task[1], QR, task[2])
            else:
                _, c, n, half = task
                oround(s - 1 if c < 0 else s, NC - 1 if c < 0 else c, n, half)
                if after_round and c >= 0:
                    after_round(c, n, half)
            for fn in extra.get(pos, ()):
                fn()

    psem = [sems.at[SEM_P + i] for i in range(7)]
    groups = [
        [cp_x(0, XC, psem[0]), cp_wq0(0, GW // 2, psem[0])],
        [cp_wq0(GW // 2, GW // 2, psem[1])],
        [cp_x(XC, XC, psem[2])],
        [cp_x(2 * XC, 2 * XC, psem[3])],
        cp_kv(0, 0, psem[4], 0, 8) + [cp_wq(0, 1, psem[4])],
        cp_kv(0, 0, psem[5], 8, 8),
        [cp_wo(0, 0, psem[6])] + cp_kv(0, 0, psem[6], 16, 16),
    ]
    for cp in sum(groups, []):
        cp.start()
    for t in (1, 2):
        for cp in cp_kv(0, t, sems.at[t]) + [cp_wo(0, t, sems.at[t]), cp_wq(0, t + 1, sems.at[t])]:
            cp.start()

    def gwait(i):
        for cp in groups[i]:
            cp.wait()

    q_buf[:, pl.ds(M_ALL, 64), :] = jnp.zeros((HG, 64, DH), BF16)
    gwait(0)
    for j in range(2):
        qproj(0, 0, XC, j)
    gwait(1)
    for j in range(2, HG):
        qproj(0, 0, XC, j)
    gwait(2)
    for j in range(HG):
        qproj(0, XC, XC, j)
    gwait(3)
    for r0 in (2 * XC, 3 * XC):
        for j in range(HG):
            qproj(0, r0, XC, j)
    gwait(4)
    step(0, ORDER_FIRST, before_k={4: lambda: gwait(5), 8: lambda: gwait(6)})
    cp_xb.start()

    def issue(t):
        sem = sems.at[slot(t)]

        @pl.when(t < NG)
        def _():
            for cp in cp_kv(0, t, sem) + [cp_wo(0, t, sem)]:
                cp.start()

        @pl.when(jnp.logical_and(t >= NG, t < NSTEP))
        def _():
            for cp in cp_kv(1, t, sem) + [cp_wo(1, t, sem)]:
                cp.start()

        @pl.when(t + 1 < NG)
        def _():
            cp_wq(0, t + 1, sem).start()

        @pl.when(jnp.logical_and(t + 1 >= NG, t + 1 < NSTEP))
        def _():
            cp_wq(1, t + 1, sem).start()

    def body(s, carry):
        wait_step(s)

        @pl.when(s == NG - 1)
        def _():
            cp_xb.wait()

        p0 = jnp.maximum(s - NG, 0) * 7
        fins = {FIN_AT + k: (lambda k=k: fin_slab(0, jnp.minimum(p0 + k, 2 * MQ // 8 - 1))) for k in range(7)}
        step(s, ORDER_MID, after_k=fins)
        issue(s + 2)
        return carry

    lax.fori_loop(1, NSTEP - 1, body, 0)

    outs = []

    def write_out(br, r0, nr, c0, nc):
        cp = pltpu.make_async_copy(stage.at[br, pl.ds(r0, nr), pl.ds(c0, nc)],
                                   o_hbm.at[pl.ds(r0, nr), pl.ds(br * D + c0, nc)], sems.at[SEM_O])
        outs.append(cp)
        cp.start()

    def after_round(c, n, half):
        for i in OUTER:
            if LAST_USE[i] != n:
                continue
            done = [blk for blk, terms in C_TERMS.items() if [k for k in OUTER if k in dict(terms)][-1] == i]
            if half is None:
                fold(1, c, i, 0, MQ)
                for r1, c1 in done:
                    write_out(1, c * MC + r1 * 2 * MQ, 2 * MQ, c1 * 2 * DH, 2 * DH)
            else:
                nr = MQ // 4 if (half == 1 and n == NR - 1) else MQ // 2
                for r in range(half * (MQ // 2), (half + 1) * (MQ // 2), nr):
                    fold(1, c, i, r, nr)
                    for r1, c1 in done:
                        for r2 in range(2):
                            write_out(1, c * MC + (2 * r1 + r2) * MQ + r, nr, c1 * 2 * DH, 2 * DH)

    write_out(0, 0, M_ALL, 0, D)
    wait_step(NSTEP - 1, with_wq=False)
    step(NSTEP - 1, ORDER_LAST, after_round=after_round)
    for cp in outs:
        cp.wait()


@jax.jit
def pallas_concat_heads__gqa_block_cached__gqa_block_cached__near_ridge_kernel(
    A_x: jax.Array,
    A_k_cache: jax.Array,
    A_v_cache: jax.Array,
    A_wq: jax.Array,
    A_wo: jax.Array,
    B_x: jax.Array,
    B_k_cache: jax.Array,
    B_v_cache: jax.Array,
    B_wq: jax.Array,
    B_wo: jax.Array,
):
    hbm = pl.BlockSpec(memory_space=pl.ANY)
    out = pl.pallas_call(
        _kernel,
        in_specs=[hbm] * 10,
        out_specs=hbm,
        out_shape=jax.ShapeDtypeStruct((M_ALL, 2 * D), BF16),
        scratch_shapes=[
            pltpu.VMEM((2, M_ALL, D), BF16),
            pltpu.VMEM((NRING, D, GW), BF16),
            pltpu.VMEM((NRING, GW, D), BF16),
            pltpu.VMEM((NRING, B, HG, SK, DH), BF16),
            pltpu.VMEM((NRING, B, HG, SK, DH), BF16),
            pltpu.VMEM((HG, M_ALL + 64, DH), BF16),
            pltpu.VMEM((NC, 4, HG, MQ, DH), F32),
            pltpu.VMEM((2, HG, SK, DH), F32),
            pltpu.VMEM((7, 7, DH, DH), BF16),
            pltpu.VMEM((2, NC, 7, 4, MQ, DH), F32),
            pltpu.VMEM((4, 2, MQ, 2 * DH), F32),
            pltpu.VMEM((2, M_ALL, D), BF16),
            pltpu.SemaphoreType.DMA((NSEM,)),
        ],
        compiler_params=pltpu.CompilerParams(
            vmem_limit_bytes=100 * 1024 * 1024,
            disable_bounds_checks=True,
            disable_semaphore_checks=True,
        ),
    )(A_x.reshape(M_ALL, D), A_k_cache, A_v_cache, A_wq, A_wo,
      B_x.reshape(M_ALL, D), B_k_cache, B_v_cache, B_wq, B_wo)
    return out.reshape(B, SQ, 2 * D)
```

```python
import math

import jax
import jax.numpy as jnp
from jax import lax
import jax.experimental.pallas as pl
import jax.experimental.pallas.tpu as pltpu

F32 = jnp.float32
BF16 = jnp.bfloat16

B, SQ, D = 32, 48, 512
H, SK, DH = 32, 48, 128
M_ALL = B * SQ
HG = 4
NG = H // HG
NSTEP = 2 * NG
GW = HG * DH
NPAIR = B // 2
NC = 2
MC = M_ALL // NC
MQ = MC // 4
QR = 192
XC = 384
C_EXP = float(DH ** -0.5) * math.log2(math.e)

NRING = 4
SEM_P = NRING
SEM_XB = SEM_P
SEM_O = SEM_P + 1
NSEM = SEM_P + 7

L_TERMS = {1: ((0, 0, 1), (1, 1, 1)), 2: ((1, 0, 1), (1, 1, 1)), 3: ((0, 0, 1),), 4: ((1, 1, 1),),
           5: ((0, 0, 1), (0, 1, 1)), 6: ((1, 0, 1), (0, 0, -1)), 7: ((0, 1, 1), (1, 1, -1))}
R_TERMS = {1: ((0, 0, 1), (1, 1, 1)), 2: ((0, 0, 1),), 3: ((0, 1, 1), (1, 1, -1)), 4: ((1, 0, 1), (0, 0, -1)),
           5: ((1, 1, 1),), 6: ((0, 0, 1), (0, 1, 1)), 7: ((1, 0, 1), (1, 1, 1))}
C_TERMS = {(0, 0): ((1, 1), (4, 1), (5, -1), (7, 1)), (0, 1): ((3, 1), (5, 1)),
           (1, 0): ((2, 1), (4, 1)), (1, 1): ((1, 1), (2, -1), (3, 1), (6, 1))}
SWAP = {1: 0, 2: 1, 3: 0, 4: 0, 5: 1, 6: 1, 7: 1}
OUTER = (2, 4, 3, 5, 1, 7, 6)

ROUNDS = []
for _i, _stray in zip(OUTER[:5], ((7, 1), (7, 7), (7, 6), (6, 1), (6, 7))):
    ROUNDS.append([(_i, _j) for _j in (3, 5, 2, 4)])
    ROUNDS.append([(_i, _j) for _j in (1, 7, 6)] + [_stray])
ROUNDS += [[(7, _j) for _j in (3, 5, 2, 4)], [(6, 6)], [(6, _j) for _j in (3, 5, 2, 4)]]
NR = len(ROUNDS)
FIRST_USE = {i: min(n for n, r in enumerate(ROUNDS) if any(p[0] == i for p in r)) for i in OUTER}
LAST_USE = {i: max(n for n, r in enumerate(ROUNDS) if any(p[0] == i for p in r)) for i in OUTER}
UPDATES = []
_seen = set()
for _r in ROUNDS:
    _u = []
    for _i in dict.fromkeys(p[0] for p in _r):
        for _blk, _terms in C_TERMS.items():
            _t = sorted(((j, sg) for (j, sg) in _terms if (_i, j) in _r), key=lambda e: -e[1])
            if _t:
                _u.append((_i, _blk, _t, (_i, _blk) not in _seen))
                _seen.add((_i, _blk))
    UPDATES.append(_u)

ORDER_FIRST = "kkqqpp" + "kqqp" * 7 + "kqqop" + "kqqoop" * 6 + "q"
ORDER_MID = "ckkqqpop" + "".join("kqq" + "o" * n + "p" for n in (2, 2, 1, 2, 2, 2, 1, 2, 2, 2, 1, 2, 2, 2)) + "q"
ORDER_LAST = "ckookpkopkopkpkopoooopkokopkpokooopokpokpkopokpoopkkoopop" + "o" * 19
N_HALVED = 5


def _comb(terms, blk):
    if len(terms) == 1:
        return blk(terms[0][0], terms[0][1])
    (r0, c0, _), (r1, c1, sg) = terms
    a, b = blk(r0, c0), blk(r1, c1)
    return a + b if sg > 0 else a - b


def _lin(terms, get):
    val = get(terms[0][0])
    for k, sg in terms[1:]:
        val = val + get(k) if sg > 0 else val - get(k)
    return val


def _lazy(fn):
    cache = {}

    def get(*k):
        if k not in cache:
            cache[k] = fn(*k)
        return cache[k]
    return get


def _dot(a, b):
    return jnp.dot(a, b, preferred_element_type=F32)


def _col_reduce(x, op, red):
    acc = x[0:8]
    for r in range(8, x.shape[0], 8):
        acc = op(acc, x[r:r + 8])
    return red(acc, axis=0, keepdims=True)


def _kernel(ax, ak, av, awq, awo, bx, bk, bv, bwq, bwo, o_hbm,
            x_buf, wq_buf, wo_buf, k_buf, v_buf, q_buf, o_buf, s_buf, r_buf, acc, c_buf, stage, sems):
    src = ((ax, ak, av, awq, awo), (bx, bk, bv, bwq, bwo))

    def slot(s):
        return s % NRING if isinstance(s, int) else jnp.bitwise_and(s, NRING - 1)

    def branch(s):
        return s // NG if isinstance(s, int) else (s >= NG).astype(jnp.int32)

    def col0(g):
        return g * GW if isinstance(g, int) else pl.multiple_of(g * GW, GW)

    def cp_wq(br, s, sem):
        return pltpu.make_async_copy(src[br][3].at[:, pl.ds(col0(s - br * NG), GW)], wq_buf.at[slot(s)], sem)

    def cp_wo(br, s, sem):
        return pltpu.make_async_copy(src[br][4].at[pl.ds(col0(s - br * NG), GW), :], wo_buf.at[slot(s)], sem)

    def cp_kv(br, s, sem, b0=0, nb=B):
        heads, rows = pl.ds((s - br * NG) * HG, HG), pl.ds(b0, nb)
        return [pltpu.make_async_copy(src[br][1].at[rows, heads], k_buf.at[slot(s), rows], sem),
                pltpu.make_async_copy(src[br][2].at[rows, heads], v_buf.at[slot(s), rows], sem)]

    def cp_x(r0, nr, sem):
        return pltpu.make_async_copy(ax.at[pl.ds(r0, nr)], x_buf.at[0, pl.ds(r0, nr)], sem)

    def cp_wq0(c0, nc, sem):
        return pltpu.make_async_copy(awq.at[:, pl.ds(c0, nc)], wq_buf.at[0, :, pl.ds(c0, nc)], sem)

    cp_xb = pltpu.make_async_copy(bx, x_buf.at[1], sems.at[SEM_XB])

    def wait_step(s, with_wq=True):
        bufs = [k_buf.at[slot(s)], v_buf.at[slot(s)], wo_buf.at[slot(s)]]
        if with_wq:
            bufs.append(wq_buf.at[slot(s + 1)])
        for buf in bufs:
            pltpu.make_async_copy(buf, buf, sems.at[slot(s)]).wait()

    def qproj(s, r0, nr, j):
        x = x_buf[branch(s), pl.ds(r0, nr), :]
        w = wq_buf[slot(s), :, pl.ds(j * DH, DH)]
        q_buf[j, pl.ds(r0, nr), :] = _dot(x, w).astype(BF16)

    def wo_tile(s, i, r1, c1, r2, c2):
        return wo_buf[slot(s), pl.ds((2 * r1 + r2) * DH, DH), pl.ds((2 * c1 + (c2 ^ SWAP[i])) * DH, DH)]

    def wo_outer(s):
        return _lazy(lambda i, r2, c2: _comb(R_TERMS[i], lambda r1, c1: wo_tile(s, i, r1, c1, r2, c2).astype(F32)))

    def plain(i, j):
        return len(R_TERMS[i]) == 1 and len(R_TERMS[j]) == 1

    def r_prep(s, i):
        outer = wo_outer(s)
        for j in range(1, 8):
            if not plain(i, j):
                r_buf[i - 1, j - 1] = _comb(R_TERMS[j], lambda r2, c2: outer(i, r2, c2)).astype(BF16)

    def fin_slab(br, p, r2):
        c = (p >= MQ // 8).astype(jnp.int32)
        r0 = pl.multiple_of(p * 8 - c * MQ, 8)
        m = _lazy(lambda k, c2: acc[br, c, k - 1, 2 * r2 + c2, pl.ds(r0, 8), :])
        for (r1, c1), terms in C_TERMS.items():
            val = jnp.concatenate([_lin(terms, lambda k: m(k, c2)) for c2 in range(2)], axis=1)
            row = pl.multiple_of(c * MC + (2 * r1 + r2) * MQ + r0, 8)
            stage[br, pl.ds(row, 8), pl.ds(c1 * 2 * DH, 2 * DH)] = val.astype(BF16)

    def fold(br, c, i, row0, nrows):
        for r0 in range(row0, row0 + nrows, SQ):
            rows = pl.ds(r0, SQ)
            for r2 in range(2):
                n = jnp.concatenate([acc[br, c, i - 1, 2 * r2 + c2, rows, :] for c2 in range(2)], axis=1)
                for (r1, c1), terms in C_TERMS.items():
                    order = [k for k in OUTER if k in dict(terms)]
                    if i not in order:
                        continue
                    pos = dict(terms)[i] > 0
                    idx = (2 * r1 + c1, r2, rows, slice(None))
                    if i == order[0]:
                        val = n if pos else -n
                    else:
                        val = c_buf[idx] + n if pos else c_buf[idx] - n
                    if i == order[-1]:
                        stage[br, pl.ds(c * MC + (2 * r1 + r2) * MQ + r0, SQ), pl.ds(c1 * 2 * DH, 2 * DH)] = val.astype(BF16)
                    else:
                        c_buf[idx] = val

    first_half = lax.broadcasted_iota(jnp.int32, (SK, DH), 1) < SQ

    def step(s, order, before_k=None, after_round=None, after_k=None):
        first, last = order is ORDER_FIRST, order is ORDER_LAST
        static = isinstance(s, int)
        sl = slot(s)
        pt, mx = {}, {}

        def scores(g):
            for j in range(HG):
                q2 = q_buf[j, pl.ds(2 * g * SQ, DH), :]
                k2 = jnp.concatenate([k_buf[sl, 2 * g + r, j, pl.ds(r0, 16), :]
                                      for r0 in range(0, SK, 16) for r in range(2)], axis=0)
                st = lax.dot_general(k2, q2, (((1,), (1,)), ((), ())), preferred_element_type=F32)
                top = jnp.concatenate([st[r0:r0 + 16] for r0 in range(0, 2 * SK, 32)], axis=0)
                bot = jnp.concatenate([st[r0 + 16:r0 + 32] for r0 in range(0, 2 * SK, 32)], axis=0)
                sc = jnp.where(first_half, top, bot)
                mx[(g, j)] = _col_reduce(sc, jnp.maximum, jnp.max)
                s_buf[g % 2, j] = sc

        def softmax(g):
            for j in range(HG):
                p = jnp.exp2((s_buf[g % 2, j] - mx[(g, j)]) * C_EXP)
                p = p * pl.reciprocal(_col_reduce(p, jnp.add, jnp.sum), approx=True)
                pt[(g, j)] = p[:, :2 * SQ].astype(BF16).T

        def pv(g):
            c, blk, half = g // 8, (g // 2) % 4, g % 2
            for r in range(2):
                for j in range(HG):
                    o_buf[c, blk, j, pl.ds((2 * half + r) * SQ, SQ), :] = _dot(
                        pt[(g, j)][r * SQ:(r + 1) * SQ], v_buf[sl, 2 * g + r, j])

        def oround(sa, c, n, half):
            init = sa % NG == 0 if static else jnp.bitwise_and(sa, NG - 1) == 0
            br = branch(sa)

            def rows(part):
                if half is not None:
                    return pl.ds(half * (MQ // 2), MQ // 2)
                return slice(None) if part is None else pl.ds(part * (MQ // 4), MQ // 4)

            raw = _lazy(lambda blk, j, part: o_buf[c, blk, j, rows(part), :])
            lin_ = _lazy(lambda i, r2, c2, part: _comb(L_TERMS[i], lambda r1, c1: raw(2 * r1 + r2, 2 * c1 + c2, part)))
            rin = wo_outer(sa)
            parts = [None] if len(ROUNDS[n]) == 4 else range(4)
            res = {}
            for part in parts:
                for i, j in ROUNDS[n]:
                    lhs = _comb(L_TERMS[j], lambda r2, c2: lin_(i, r2, c2, part)).astype(BF16)
                    if plain(i, j):
                        rhs = wo_tile(sa, i, *R_TERMS[i][0][:2], *R_TERMS[j][0][:2])
                    elif first:
                        w = _comb(R_TERMS[j], lambda r2, c2: rin(i, r2, c2))
                        rhs = w.astype(BF16)
                        if part in (None, 0):
                            r_buf[i - 1, j - 1] = (w + 0.0).astype(BF16)
                    else:
                        rhs = r_buf[i - 1, j - 1]
                    res[(i, j, part)] = _dot(lhs, rhs)
            for part in parts:
                for i, (r2, c2), terms, first_touch in UPDATES[n]:
                    val = _lin(terms, lambda j: res[(i, j, part)])
                    idx = (br, c, i - 1, 2 * r2 + (c2 ^ SWAP[i]), rows(part), slice(None))
                    if not first_touch:
                        acc[idx] = acc[idx] + val
                    elif static:
                        acc[idx] = val if init else acc[idx] + val
                    else:
                        acc[idx] = jnp.where(init, 0.0, acc[idx]) + val

        qpieces = [(r0, j) for r0 in range(0, M_ALL, QR) for j in range(HG)]
        carried = qpieces.pop()
        rounds = [] if first else [(-1, n, None) for n in range(NR)]
        rounds += [(0, n, None) for n in range(NR)]
        if last:
            tail = range(NR - N_HALVED, NR)
            rounds += [(1, n, None) for n in range(NR) if n not in tail or len(ROUNDS[n]) != 4]
            rounds += [(1, n, h) for h in range(2) for n in tail if len(ROUNDS[n]) == 4]
        count = dict.fromkeys("kpqco", 0)
        tasks = []
        for t in order:
            n = count[t]
            count[t] += 1
            if t == "k":
                assert n - count["p"] < 2 and (first or count["c"] == 1)
                tasks.append(("k", n))
            elif t == "p":
                assert n < count["k"] and (first or n < 8 or count["o"] >= NR)
                tasks.append(("p", n))
            elif t == "q":
                assert qpieces[n][0] + QR <= count["k"] * 2 * SQ
                tasks.append(("q",) + qpieces[n])
            elif t == "c":
                tasks.append(("c",) + carried)
            else:
                assert count["p"] >= 8 * (rounds[n][0] + 1)
                tasks.append(("o",) + rounds[n])
        assert count["k"] == count["p"] == NPAIR and count["o"] == len(rounds)
        assert count["q"] == (0 if last else len(qpieces)) and count["c"] == (0 if first else 1)

        extra = {}
        for g in range(NPAIR):
            pos = min(tasks.index(("k", g)) + 1, tasks.index(("p", g)) - 1)
            extra.setdefault(pos, []).append(lambda g=g: softmax(g))
        if not first:
            for i in OUTER:
                pos = tasks.index(("o", -1, LAST_USE[i], None))
                assert pos < tasks.index(("o", 0, FIRST_USE[i], None))
                extra.setdefault(pos, []).append(lambda i=i: r_prep(s, i))
        for g, fn in (after_k or {}).items():
            extra.setdefault(tasks.index(("k", g)) + 1, []).append(fn)

        for pos, task in enumerate(tasks):
            if task[0] == "k":
                if before_k and task[1] in before_k:
                    before_k[task[1]]()
                scores(task[1])
            elif task[0] == "p":
                pv(task[1])
            elif task[0] == "q":
                qproj(s + 1, task[1], QR, task[2])
            elif task[0] == "c":
                qproj(s, task[1], QR, task[2])
            else:
                _, c, n, half = task
                oround(s - 1 if c < 0 else s, NC - 1 if c < 0 else c, n, half)
                if after_round and c >= 0:
                    after_round(c, n, half)
            for fn in extra.get(pos, ()):
                fn()

    psem = [sems.at[SEM_P + i] for i in range(7)]
    groups = [
        [cp_x(0, XC, psem[0]), cp_wq0(0, GW // 2, psem[0])],
        [cp_wq0(GW // 2, GW // 2, psem[1])],
        [cp_x(XC, XC, psem[2])],
        [cp_x(2 * XC, 2 * XC, psem[3])],
        cp_kv(0, 0, psem[4], 0, 8) + [cp_wq(0, 1, psem[4])],
        cp_kv(0, 0, psem[5], 8, 8),
        [cp_wo(0, 0, psem[6])] + cp_kv(0, 0, psem[6], 16, 16),
    ]
    for cp in sum(groups, []):
        cp.start()
    for t in (1, 2):
        for cp in cp_kv(0, t, sems.at[t]) + [cp_wo(0, t, sems.at[t]), cp_wq(0, t + 1, sems.at[t])]:
            cp.start()

    def gwait(i):
        for cp in groups[i]:
            cp.wait()

    q_buf[:, pl.ds(M_ALL, 64), :] = jnp.zeros((HG, 64, DH), BF16)
    gwait(0)
    for j in range(2):
        qproj(0, 0, XC, j)
    gwait(1)
    for j in range(2, HG):
        qproj(0, 0, XC, j)
    gwait(2)
    for j in range(HG):
        qproj(0, XC, XC, j)
    gwait(3)
    for r0 in (2 * XC, 3 * XC):
        for j in range(HG):
            qproj(0, r0, XC, j)
    gwait(4)
    step(0, ORDER_FIRST, before_k={4: lambda: gwait(5), 8: lambda: gwait(6)})
    cp_xb.start()

    def issue(t):
        sem = sems.at[slot(t)]

        @pl.when(t < NG)
        def _():
            for cp in cp_kv(0, t, sem) + [cp_wo(0, t, sem)]:
                cp.start()

        @pl.when(jnp.logical_and(t >= NG, t < NSTEP))
        def _():
            for cp in cp_kv(1, t, sem) + [cp_wo(1, t, sem)]:
                cp.start()

        @pl.when(t + 1 < NG)
        def _():
            cp_wq(0, t + 1, sem).start()

        @pl.when(jnp.logical_and(t + 1 >= NG, t + 1 < NSTEP))
        def _():
            cp_wq(1, t + 1, sem).start()

    def body(s, carry):
        wait_step(s)

        @pl.when(s == NG - 1)
        def _():
            cp_xb.wait()

        p0 = jnp.maximum(s - NG, 0) * 7
        fins = {2 + k: (lambda k=k: fin_slab(0, jnp.minimum(p0 + k // 2, 2 * MQ // 8 - 1), k % 2)) for k in range(14)}
        step(s, ORDER_MID, after_k=fins)
        issue(s + 2)
        return carry

    lax.fori_loop(1, NSTEP - 1, body, 0)

    outs = []

    def write_out(br, r0, nr, c0, nc):
        cp = pltpu.make_async_copy(stage.at[br, pl.ds(r0, nr), pl.ds(c0, nc)],
                                   o_hbm.at[pl.ds(r0, nr), pl.ds(br * D + c0, nc)], sems.at[SEM_O])
        outs.append(cp)
        cp.start()

    def after_round(c, n, half):
        for i in OUTER:
            if LAST_USE[i] != n:
                continue
            done = [blk for blk, terms in C_TERMS.items() if [k for k in OUTER if k in dict(terms)][-1] == i]
            if half is None:
                fold(1, c, i, 0, MQ)
                for r1, c1 in done:
                    write_out(1, c * MC + r1 * 2 * MQ, 2 * MQ, c1 * 2 * DH, 2 * DH)
            else:
                nr = MQ // 4 if (half == 1 and n == NR - 1) else MQ // 2
                for r in range(half * (MQ // 2), (half + 1) * (MQ // 2), nr):
                    fold(1, c, i, r, nr)
                    for r1, c1 in done:
                        for r2 in range(2):
                            write_out(1, c * MC + (2 * r1 + r2) * MQ + r, nr, c1 * 2 * DH, 2 * DH)

    write_out(0, 0, M_ALL, 0, D)
    wait_step(NSTEP - 1, with_wq=False)
    step(NSTEP - 1, ORDER_LAST, after_round=after_round)
    for cp in outs:
        cp.wait()


@jax.jit
def pallas_concat_heads__gqa_block_cached__gqa_block_cached__near_ridge_kernel(
    A_x: jax.Array,
    A_k_cache: jax.Array,
    A_v_cache: jax.Array,
    A_wq: jax.Array,
    A_wo: jax.Array,
    B_x: jax.Array,
    B_k_cache: jax.Array,
    B_v_cache: jax.Array,
    B_wq: jax.Array,
    B_wo: jax.Array,
):
    hbm = pl.BlockSpec(memory_space=pl.ANY)
    out = pl.pallas_call(
        _kernel,
        in_specs=[hbm] * 10,
        out_specs=hbm,
        out_shape=jax.ShapeDtypeStruct((M_ALL, 2 * D), BF16),
        scratch_shapes=[
            pltpu.VMEM((2, M_ALL, D), BF16),
            pltpu.VMEM((NRING, D, GW), BF16),
            pltpu.VMEM((NRING, GW, D), BF16),
            pltpu.VMEM((NRING, B, HG, SK, DH), BF16),
            pltpu.VMEM((NRING, B, HG, SK, DH), BF16),
            pltpu.VMEM((HG, M_ALL + 64, DH), BF16),
            pltpu.VMEM((NC, 4, HG, MQ, DH), F32),
            pltpu.VMEM((2, HG, SK, DH), F32),
            pltpu.VMEM((7, 7, DH, DH), BF16),
            pltpu.VMEM((2, NC, 7, 4, MQ, DH), F32),
            pltpu.VMEM((4, 2, MQ, 2 * DH), F32),
            pltpu.VMEM((2, M_ALL, D), BF16),
            pltpu.SemaphoreType.DMA((NSEM,)),
        ],
        compiler_params=pltpu.CompilerParams(
            vmem_limit_bytes=100 * 1024 * 1024,
            disable_bounds_checks=True,
            disable_semaphore_checks=True,
        ),
    )(A_x.reshape(M_ALL, D), A_k_cache, A_v_cache, A_wq, A_wo,
      B_x.reshape(M_ALL, D), B_k_cache, B_v_cache, B_wq, B_wo)
    return out.reshape(B, SQ, 2 * D)
```

```python
import math

import jax
import jax.numpy as jnp
from jax import lax
import jax.experimental.pallas as pl
import jax.experimental.pallas.tpu as pltpu

F32 = jnp.float32
BF16 = jnp.bfloat16

B, SQ, D = 32, 48, 512
H, SK, DH = 32, 48, 128
M_ALL = B * SQ
HG = 4
NG = H // HG
NSTEP = 2 * NG
GW = HG * DH
NPAIR = B // 2
NC = 2
MC = M_ALL // NC
MQ = MC // 4
QR = 192
XC = 384
C_EXP = float(DH ** -0.5) * math.log2(math.e)

NRING = 4
SEM_P = NRING
SEM_XB = SEM_P
SEM_O = SEM_P + 1
NSEM = SEM_P + 7

L_TERMS = {1: ((0, 0, 1), (1, 1, 1)), 2: ((1, 0, 1), (1, 1, 1)), 3: ((0, 0, 1),), 4: ((1, 1, 1),),
           5: ((0, 0, 1), (0, 1, 1)), 6: ((1, 0, 1), (0, 0, -1)), 7: ((0, 1, 1), (1, 1, -1))}
R_TERMS = {1: ((0, 0, 1), (1, 1, 1)), 2: ((0, 0, 1),), 3: ((0, 1, 1), (1, 1, -1)), 4: ((1, 0, 1), (0, 0, -1)),
           5: ((1, 1, 1),), 6: ((0, 0, 1), (0, 1, 1)), 7: ((1, 0, 1), (1, 1, 1))}
C_TERMS = {(0, 0): ((1, 1), (4, 1), (5, -1), (7, 1)), (0, 1): ((3, 1), (5, 1)),
           (1, 0): ((2, 1), (4, 1)), (1, 1): ((1, 1), (2, -1), (3, 1), (6, 1))}
SWAP = {1: 0, 2: 1, 3: 0, 4: 0, 5: 1, 6: 1, 7: 1}
OUTER = (2, 4, 3, 5, 1, 7, 6)

ROUNDS = []
for _i, _stray in zip(OUTER[:5], ((7, 1), (7, 7), (7, 6), (6, 1), (6, 7))):
    ROUNDS.append([(_i, _j) for _j in (3, 5, 2, 4)])
    ROUNDS.append([(_i, _j) for _j in (1, 7, 6)] + [_stray])
ROUNDS += [[(7, _j) for _j in (3, 5, 2, 4)], [(6, 6)], [(6, _j) for _j in (3, 5, 2, 4)]]
NR = len(ROUNDS)
FIRST_USE = {i: min(n for n, r in enumerate(ROUNDS) if any(p[0] == i for p in r)) for i in OUTER}
LAST_USE = {i: max(n for n, r in enumerate(ROUNDS) if any(p[0] == i for p in r)) for i in OUTER}
UPDATES = []
_seen = set()
for _r in ROUNDS:
    _u = []
    for _i in dict.fromkeys(p[0] for p in _r):
        for _blk, _terms in C_TERMS.items():
            _t = sorted(((j, sg) for (j, sg) in _terms if (_i, j) in _r), key=lambda e: -e[1])
            if _t:
                _u.append((_i, _blk, _t, (_i, _blk) not in _seen))
                _seen.add((_i, _blk))
    UPDATES.append(_u)

ORDER_FIRST = "kkqqpp" + "kqqp" * 7 + "kqqop" + "kqqoop" * 6 + "q"
ORDER_MID = "ckkqqpop" + "".join("kqq" + "o" * n + "p" for n in (2, 2, 1, 2, 2, 2, 1, 2, 2, 2, 1, 2, 2, 2)) + "q"
ORDER_LAST = "ckookpkopkopkpkopoooopkokopkpokooopokpokpkopokpoopkkoopop" + "o" * 19
N_HALVED = 5


def _comb(terms, blk):
    if len(terms) == 1:
        return blk(terms[0][0], terms[0][1])
    (r0, c0, _), (r1, c1, sg) = terms
    a, b = blk(r0, c0), blk(r1, c1)
    return a + b if sg > 0 else a - b


def _lin(terms, get):
    val = get(terms[0][0])
    for k, sg in terms[1:]:
        val = val + get(k) if sg > 0 else val - get(k)
    return val


def _lazy(fn):
    cache = {}

    def get(*k):
        if k not in cache:
            cache[k] = fn(*k)
        return cache[k]
    return get


def _dot(a, b):
    return jnp.dot(a, b, preferred_element_type=F32)


def _col_reduce(x, op, red):
    acc = x[0:8]
    for r in range(8, x.shape[0], 8):
        acc = op(acc, x[r:r + 8])
    return red(acc, axis=0, keepdims=True)


def _kernel(ax, ak, av, awq, awo, bx, bk, bv, bwq, bwo, o_hbm,
            x_buf, wq_buf, wo_buf, k_buf, v_buf, q_buf, o_buf, s_buf, r_buf, acc, c_buf, stage, sems):
    src = ((ax, ak, av, awq, awo), (bx, bk, bv, bwq, bwo))

    def slot(s):
        return s % NRING if isinstance(s, int) else jnp.bitwise_and(s, NRING - 1)

    def branch(s):
        return s // NG if isinstance(s, int) else (s >= NG).astype(jnp.int32)

    def col0(g):
        return g * GW if isinstance(g, int) else pl.multiple_of(g * GW, GW)

    def cp_wq(br, s, sem):
        return pltpu.make_async_copy(src[br][3].at[:, pl.ds(col0(s - br * NG), GW)], wq_buf.at[slot(s)], sem)

    def cp_wo(br, s, sem):
        return pltpu.make_async_copy(src[br][4].at[pl.ds(col0(s - br * NG), GW), :], wo_buf.at[slot(s)], sem)

    def cp_kv(br, s, sem, b0=0, nb=B):
        heads, rows = pl.ds((s - br * NG) * HG, HG), pl.ds(b0, nb)
        return [pltpu.make_async_copy(src[br][1].at[rows, heads], k_buf.at[slot(s), rows], sem),
                pltpu.make_async_copy(src[br][2].at[rows, heads], v_buf.at[slot(s), rows], sem)]

    def cp_x(r0, nr, sem):
        return pltpu.make_async_copy(ax.at[pl.ds(r0, nr)], x_buf.at[0, pl.ds(r0, nr)], sem)

    def cp_wq0(c0, nc, sem):
        return pltpu.make_async_copy(awq.at[:, pl.ds(c0, nc)], wq_buf.at[0, :, pl.ds(c0, nc)], sem)

    cp_xb = pltpu.make_async_copy(bx, x_buf.at[1], sems.at[SEM_XB])

    def wait_step(s, with_wq=True):
        bufs = [k_buf.at[slot(s)], v_buf.at[slot(s)], wo_buf.at[slot(s)]]
        if with_wq:
            bufs.append(wq_buf.at[slot(s + 1)])
        for buf in bufs:
            pltpu.make_async_copy(buf, buf, sems.at[slot(s)]).wait()

    def qproj(s, r0, nr, j):
        x = x_buf[branch(s), pl.ds(r0, nr), :]
        w = wq_buf[slot(s), :, pl.ds(j * DH, DH)]
        q_buf[j, pl.ds(r0, nr), :] = _dot(x, w).astype(BF16)

    def wo_tile(s, i, r1, c1, r2, c2):
        return wo_buf[slot(s), pl.ds((2 * r1 + r2) * DH, DH), pl.ds((2 * c1 + (c2 ^ SWAP[i])) * DH, DH)]

    def wo_outer(s):
        return _lazy(lambda i, r2, c2: _comb(R_TERMS[i], lambda r1, c1: wo_tile(s, i, r1, c1, r2, c2).astype(F32)))

    def plain(i, j):
        return len(R_TERMS[i]) == 1 and len(R_TERMS[j]) == 1

    def r_prep(s, i):
        outer = wo_outer(s)
        for j in range(1, 8):
            if not plain(i, j):
                r_buf[i - 1, j - 1] = _comb(R_TERMS[j], lambda r2, c2: outer(i, r2, c2)).astype(BF16)

    def fin_slab(br, p, r2):
        c = (p >= MQ // 8).astype(jnp.int32)
        r0 = pl.multiple_of(p * 8 - c * MQ, 8)
        m = _lazy(lambda k, c2: acc[br, c, k - 1, 2 * r2 + c2, pl.ds(r0, 8), :])
        for (r1, c1), terms in C_TERMS.items():
            val = jnp.concatenate([_lin(terms, lambda k: m(k, c2)) for c2 in range(2)], axis=1)
            row = pl.multiple_of(c * MC + (2 * r1 + r2) * MQ + r0, 8)
            stage[br, pl.ds(row, 8), pl.ds(c1 * 2 * DH, 2 * DH)] = val.astype(BF16)

    def fold(br, c, i, row0, nrows):
        for r0 in range(row0, row0 + nrows, SQ):
            rows = pl.ds(r0, SQ)
            for r2 in range(2):
                n = jnp.concatenate([acc[br, c, i - 1, 2 * r2 + c2, rows, :] for c2 in range(2)], axis=1)
                for (r1, c1), terms in C_TERMS.items():
                    order = [k for k in OUTER if k in dict(terms)]
                    if i not in order:
                        continue
                    pos = dict(terms)[i] > 0
                    idx = (2 * r1 + c1, r2, rows, slice(None))
                    if i == order[0]:
                        val = n if pos else -n
                    else:
                        val = c_buf[idx] + n if pos else c_buf[idx] - n
                    if i == order[-1]:
                        stage[br, pl.ds(c * MC + (2 * r1 + r2) * MQ + r0, SQ), pl.ds(c1 * 2 * DH, 2 * DH)] = val.astype(BF16)
                    else:
                        c_buf[idx] = val

    first_half = lax.broadcasted_iota(jnp.int32, (SK, DH), 1) < SQ

    def step(s, order, before_k=None, after_round=None, after_k=None):
        first, last = order is ORDER_FIRST, order is ORDER_LAST
        static = isinstance(s, int)
        sl = slot(s)
        pt, mx = {}, {}

        def scores(g):
            for j in range(HG):
                q2 = q_buf[j, pl.ds(2 * g * SQ, DH), :]
                k2 = jnp.concatenate([k_buf[sl, 2 * g + r, j, pl.ds(r0, 16), :]
                                      for r0 in range(0, SK, 16) for r in range(2)], axis=0)
                st = lax.dot_general(k2, q2, (((1,), (1,)), ((), ())), preferred_element_type=F32)
                top = jnp.concatenate([st[r0:r0 + 16] for r0 in range(0, 2 * SK, 32)], axis=0)
                bot = jnp.concatenate([st[r0 + 16:r0 + 32] for r0 in range(0, 2 * SK, 32)], axis=0)
                sc = jnp.where(first_half, top, bot)
                mx[(g, j)] = _col_reduce(sc, jnp.maximum, jnp.max)
                s_buf[g % 2, j] = sc

        def softmax(g):
            for j in range(HG):
                p = jnp.exp2((s_buf[g % 2, j] - mx[(g, j)]) * C_EXP)
                p = p * pl.reciprocal(_col_reduce(p, jnp.add, jnp.sum), approx=True)
                pt[(g, j)] = p[:, :2 * SQ].astype(BF16).T

        def pv(g):
            c, blk, half = g // 8, (g // 2) % 4, g % 2
            for r in range(2):
                for j in range(HG):
                    o_buf[c, blk, j, pl.ds((2 * half + r) * SQ, SQ), :] = _dot(
                        pt[(g, j)][r * SQ:(r + 1) * SQ], v_buf[sl, 2 * g + r, j])

        def oround(sa, c, n, half):
            init = sa % NG == 0 if static else jnp.bitwise_and(sa, NG - 1) == 0
            br = branch(sa)

            def rows(part):
                if half is not None:
                    return pl.ds(half * (MQ // 2), MQ // 2)
                return slice(None) if part is None else pl.ds(part * (MQ // 4), MQ // 4)

            raw = _lazy(lambda blk, j, part: o_buf[c, blk, j, rows(part), :])
            lin_ = _lazy(lambda i, r2, c2, part: _comb(L_TERMS[i], lambda r1, c1: raw(2 * r1 + r2, 2 * c1 + c2, part)))
            rin = wo_outer(sa)
            parts = [None] if len(ROUNDS[n]) == 4 else range(4)
            res = {}
            for part in parts:
                for i, j in ROUNDS[n]:
                    lhs = _comb(L_TERMS[j], lambda r2, c2: lin_(i, r2, c2, part)).astype(BF16)
                    if plain(i, j):
                        rhs = wo_tile(sa, i, *R_TERMS[i][0][:2], *R_TERMS[j][0][:2])
                    elif first:
                        w = _comb(R_TERMS[j], lambda r2, c2: rin(i, r2, c2))
                        rhs = w.astype(BF16)
                        if part in (None, 0):
                            r_buf[i - 1, j - 1] = (w + 0.0).astype(BF16)
                    else:
                        rhs = r_buf[i - 1, j - 1]
                    res[(i, j, part)] = _dot(lhs, rhs)
            for part in parts:
                for i, (r2, c2), terms, first_touch in UPDATES[n]:
                    val = _lin(terms, lambda j: res[(i, j, part)])
                    idx = (br, c, i - 1, 2 * r2 + (c2 ^ SWAP[i]), rows(part), slice(None))
                    if not first_touch:
                        acc[idx] = acc[idx] + val
                    elif static:
                        acc[idx] = val if init else acc[idx] + val
                    else:
                        acc[idx] = jnp.where(init, 0.0, acc[idx]) + val

        qpieces = [(r0, j) for r0 in range(0, M_ALL, QR) for j in range(HG)]
        carried = qpieces.pop()
        rounds = [] if first else [(-1, n, None) for n in range(NR)]
        rounds += [(0, n, None) for n in range(NR)]
        if last:
            tail = range(NR - N_HALVED, NR)
            rounds += [(1, n, None) for n in range(NR) if n not in tail or len(ROUNDS[n]) != 4]
            rounds += [(1, n, h) for h in range(2) for n in tail if len(ROUNDS[n]) == 4]
        count = dict.fromkeys("kpqco", 0)
        tasks = []
        for t in order:
            n = count[t]
            count[t] += 1
            if t == "k":
                assert n - count["p"] < 2 and (first or count["c"] == 1)
                tasks.append(("k", n))
            elif t == "p":
                assert n < count["k"] and (first or n < 8 or count["o"] >= NR)
                tasks.append(("p", n))
            elif t == "q":
                assert qpieces[n][0] + QR <= count["k"] * 2 * SQ
                tasks.append(("q",) + qpieces[n])
            elif t == "c":
                tasks.append(("c",) + carried)
            else:
                assert count["p"] >= 8 * (rounds[n][0] + 1)
                tasks.append(("o",) + rounds[n])
        assert count["k"] == count["p"] == NPAIR and count["o"] == len(rounds)
        assert count["q"] == (0 if last else len(qpieces)) and count["c"] == (0 if first else 1)

        extra = {}
        for g in range(NPAIR):
            pos = min(tasks.index(("k", g)) + 1, tasks.index(("p", g)) - 1)
            extra.setdefault(pos, []).append(lambda g=g: softmax(g))
        if not first:
            for i in OUTER:
                pos = tasks.index(("o", -1, LAST_USE[i], None))
                assert pos < tasks.index(("o", 0, FIRST_USE[i], None))
                extra.setdefault(pos, []).append(lambda i=i: r_prep(s, i))
        for g, fn in (after_k or {}).items():
            extra.setdefault(tasks.index(("k", g)) + 1, []).append(fn)

        for pos, task in enumerate(tasks):
            if task[0] == "k":
                if before_k and task[1] in before_k:
                    before_k[task[1]]()
                scores(task[1])
            elif task[0] == "p":
                pv(task[1])
            elif task[0] == "q":
                qproj(s + 1, task[1], QR, task[2])
            elif task[0] == "c":
                qproj(s, task[1], QR, task[2])
            else:
                _, c, n, half = task
                oround(s - 1 if c < 0 else s, NC - 1 if c < 0 else c, n, half)
                if after_round and c >= 0:
                    after_round(c, n, half)
            for fn in extra.get(pos, ()):
                fn()

    psem = [sems.at[SEM_P + i] for i in range(7)]
    groups = [
        [cp_x(0, XC, psem[0]), cp_wq0(0, GW // 2, psem[0])],
        [cp_wq0(GW // 2, GW // 2, psem[1])],
        [cp_x(XC, XC, psem[2])],
        [cp_x(2 * XC, 2 * XC, psem[3])],
        cp_kv(0, 0, psem[4], 0, 8) + [cp_wq(0, 1, psem[4])],
        cp_kv(0, 0, psem[5], 8, 8),
        [cp_wo(0, 0, psem[6])] + cp_kv(0, 0, psem[6], 16, 16),
    ]
    for cp in sum(groups, []):
        cp.start()
    for t in (1, 2):
        for cp in cp_kv(0, t, sems.at[t]) + [cp_wo(0, t, sems.at[t]), cp_wq(0, t + 1, sems.at[t])]:
            cp.start()

    def gwait(i):
        for cp in groups[i]:
            cp.wait()

    q_buf[:, pl.ds(M_ALL, 64), :] = jnp.zeros((HG, 64, DH), BF16)
    gwait(0)
    for j in range(2):
        qproj(0, 0, XC, j)
    gwait(1)
    for j in range(2, HG):
        qproj(0, 0, XC, j)
    gwait(2)
    for j in range(HG):
        qproj(0, XC, XC, j)
    gwait(3)
    for r0 in (2 * XC, 3 * XC):
        for j in range(HG):
            qproj(0, r0, XC, j)
    gwait(4)
    step(0, ORDER_FIRST, before_k={4: lambda: gwait(5), 8: lambda: gwait(6)})
    cp_xb.start()

    def issue(t):
        sem = sems.at[slot(t)]

        @pl.when(t < NG)
        def _():
            for cp in cp_kv(0, t, sem) + [cp_wo(0, t, sem)]:
                cp.start()

        @pl.when(jnp.logical_and(t >= NG, t < NSTEP))
        def _():
            for cp in cp_kv(1, t, sem) + [cp_wo(1, t, sem)]:
                cp.start()

        @pl.when(t + 1 < NG)
        def _():
            cp_wq(0, t + 1, sem).start()

        @pl.when(jnp.logical_and(t + 1 >= NG, t + 1 < NSTEP))
        def _():
            cp_wq(1, t + 1, sem).start()

    def body(s, carry):
        wait_step(s)

        @pl.when(s == NG - 1)
        def _():
            cp_xb.wait()

        p0 = jnp.maximum(s - NG, 0) * 7
        fins = {2 + k: (lambda k=k: fin_slab(0, jnp.minimum(p0 + k // 2, 2 * MQ // 8 - 1), k % 2)) for k in range(14)}
        step(s, ORDER_MID, after_k=fins)
        issue(s + 2)
        return carry

    lax.fori_loop(1, NSTEP - 1, body, 0)

    outs = []

    def write_out(br, r0, nr, c0, nc):
        cp = pltpu.make_async_copy(stage.at[br, pl.ds(r0, nr), pl.ds(c0, nc)],
                                   o_hbm.at[pl.ds(r0, nr), pl.ds(br * D + c0, nc)], sems.at[SEM_O])
        outs.append(cp)
        cp.start()

    def after_round(c, n, half):
        for i in OUTER:
            if LAST_USE[i] != n:
                continue
            done = [blk for blk, terms in C_TERMS.items() if [k for k in OUTER if k in dict(terms)][-1] == i]
            if half is None:
                fold(1, c, i, 0, MQ)
                for r1, c1 in done:
                    write_out(1, c * MC + r1 * 2 * MQ, 2 * MQ, c1 * 2 * DH, 2 * DH)
            else:
                nr = MQ // 4 if (half == 1 and n == NR - 1) else MQ // 2
                for r in range(half * (MQ // 2), (half + 1) * (MQ // 2), nr):
                    fold(1, c, i, r, nr)
                    for r1, c1 in done:
                        for r2 in range(2):
                            write_out(1, c * MC + (2 * r1 + r2) * MQ + r, nr, c1 * 2 * DH, 2 * DH)

    write_out(0, 0, M_ALL, 0, D)
    wait_step(NSTEP - 1, with_wq=False)
    step(NSTEP - 1, ORDER_LAST, after_round=after_round)
    for cp in outs:
        cp.wait()


def _compiler_params():
    base = dict(vmem_limit_bytes=100 * 1024 * 1024, disable_bounds_checks=True)
    try:
        return pltpu.CompilerParams(disable_semaphore_checks=True, **base)
    except TypeError:
        return pltpu.CompilerParams(**base)


@jax.jit
def pallas_concat_heads__gqa_block_cached__gqa_block_cached__near_ridge_kernel(
    A_x: jax.Array,
    A_k_cache: jax.Array,
    A_v_cache: jax.Array,
    A_wq: jax.Array,
    A_wo: jax.Array,
    B_x: jax.Array,
    B_k_cache: jax.Array,
    B_v_cache: jax.Array,
    B_wq: jax.Array,
    B_wo: jax.Array,
):
    hbm = pl.BlockSpec(memory_space=pl.ANY)
    out = pl.pallas_call(
        _kernel,
        in_specs=[hbm] * 10,
        out_specs=hbm,
        out_shape=jax.ShapeDtypeStruct((M_ALL, 2 * D), BF16),
        scratch_shapes=[
            pltpu.VMEM((2, M_ALL, D), BF16),
            pltpu.VMEM((NRING, D, GW), BF16),
            pltpu.VMEM((NRING, GW, D), BF16),
            pltpu.VMEM((NRING, B, HG, SK, DH), BF16),
            pltpu.VMEM((NRING, B, HG, SK, DH), BF16),
            pltpu.VMEM((HG, M_ALL + 64, DH), BF16),
            pltpu.VMEM((NC, 4, HG, MQ, DH), F32),
            pltpu.VMEM((2, HG, SK, DH), F32),
            pltpu.VMEM((7, 7, DH, DH), BF16),
            pltpu.VMEM((2, NC, 7, 4, MQ, DH), F32),
            pltpu.VMEM((4, 2, MQ, 2 * DH), F32),
            pltpu.VMEM((2, M_ALL, D), BF16),
            pltpu.SemaphoreType.DMA((NSEM,)),
        ],
        compiler_params=_compiler_params(),
    )(A_x.reshape(M_ALL, D), A_k_cache, A_v_cache, A_wq, A_wo,
      B_x.reshape(M_ALL, D), B_k_cache, B_v_cache, B_wq, B_wo)
    return out.reshape(B, SQ, 2 * D)
```
